```python
import jax
import jax.numpy as jnp

def _softmax(x, axis=-1):
    return jax.nn.softmax(x, axis=axis)

def _gelu(x):
    return jax.nn.gelu(x, approximate=True)

def _silu(x):
    return jax.nn.silu(x)

def _sigmoid(x):
    return jax.nn.sigmoid(x)

def _layernorm(x, axis=-1, eps=1e-05):
    m = jnp.mean(x, axis=axis, keepdims=True)
    v = jnp.var(x, axis=axis, keepdims=True)
    return (x - m) / jnp.sqrt(v + eps)

def _scatter_add(tgt, idx, src, axis=0):
    return tgt.at[idx].add(src)

def _segment_sum(src, seg, n):
    return jax.ops.segment_sum(src, seg, n)

class _Rng:

    def __init__(self, key):
        self._k = key

    def _next(self):
        self._k, sub = jax.random.split(self._k)
        return sub

    def normal(self, shape):
        return jax.random.normal(self._next(), shape, dtype=jnp.bfloat16)

    def randint(self, lo, hi, shape):
        return jax.random.randint(self._next(), shape, lo, hi, dtype=jnp.int32)

    def uniform(self, shape, lo=0.0, hi=1.0):
        return jax.random.uniform(self._next(), shape, jnp.bfloat16, lo, hi)

    def permutation(self, n):
        return jax.random.permutation(self._next(), n)
kernel_name = 'gated_mix__ssm_conv_h3__memory_aug_recurrent_mem_tr__prompt'

def setup_inputs():
    _rng = _Rng(jax.random.key(int.from_bytes(__import__("os").urandom(4), "little")))
    _w = lambda a: (lambda t: t.astype(jnp.bfloat16) if jnp.issubdtype(t.dtype, jnp.floating) else t)(jnp.asarray(a))

    def _A_setup():
        B, S, D = (1, 2048, 1024)
        ks = 4
        return {'q': _w((lambda *s: _rng.normal(s) * 0.05)(B, S, D)), 'k': _w((lambda *s: _rng.normal(s) * 0.05)(B, S, D)), 'v': _w((lambda *s: _rng.normal(s) * 0.05)(B, S, D)), 'shift_k': _w((lambda *s: _rng.normal(s) * 0.05)(D, ks) * 0.5), 'ssm_k': _w((lambda *s: _rng.normal(s) * 0.05)(D, S) * (1.0 / S ** 0.5)), 'ssm_D': _w((lambda *s: _rng.normal(s) * 0.05)(D))}
    _A_in = _A_setup()

    def _B_setup():
        B, S, Dm = (1, 2048, 1024)
        H, Dh = (32, 128)
        M, seg = (8, 32)
        seg = min(seg, S)
        S = S // seg * seg
        return {'x': _w((lambda *s: _rng.normal(s) * 0.05)(B, S, Dm)), 'mem0': _w((lambda *s: _rng.normal(s) * 0.05)(B, M, Dm)), 'Wq': _w((lambda *s: _rng.normal(s) * 0.05)(Dm, H, Dh) * Dm ** (-0.5)), 'Wk': _w((lambda *s: _rng.normal(s) * 0.05)(Dm, H, Dh) * Dm ** (-0.5)), 'Wv': _w((lambda *s: _rng.normal(s) * 0.05)(Dm, H, Dh) * Dm ** (-0.5)), 'Wo': _w((lambda *s: _rng.normal(s) * 0.05)(H, Dh, Dm) * (H * Dh) ** (-0.5)), 'seg_len': seg}
    _B_in = _B_setup()
    return {'A_q': _A_in['q'], 'A_k': _A_in['k'], 'A_v': _A_in['v'], 'A_shift_k': _A_in['shift_k'], 'A_ssm_k': _A_in['ssm_k'], 'A_ssm_D': _A_in['ssm_D'], 'B_x': _B_in['x'], 'B_mem0': _B_in['mem0'], 'B_Wq': _B_in['Wq'], 'B_Wk': _B_in['Wk'], 'B_Wv': _B_in['Wv'], 'B_Wo': _B_in['Wo'], 'B_seg_len': _B_in['seg_len'], 'gate_w': _w((lambda *s: _rng.normal(s) * 0.05)(1024))}

def reference(A_q, A_k, A_v, A_shift_k, A_ssm_k, A_ssm_D, B_x, B_mem0, B_Wq, B_Wk, B_Wv, B_Wo, B_seg_len, gate_w):

    def _A_ref(q, k, v, shift_k, ssm_k, ssm_D):
        B, S, D = q.shape
        ks = shift_k.shape[-1]
        k_pad = jnp.pad(k, ((0, 0), (ks - 1, 0), (0, 0)))
        k_shift = jnp.zeros_like(k)
        for t in range(ks):
            k_shift = k_shift + k_pad[:, t:t + S, :] * shift_k[:, ks - 1 - t][None, None, :]
        kv = k_shift * v
        L = 2 * S
        kv_pad = jnp.pad(kv, ((0, 0), (0, S), (0, 0)))
        kf_pad = jnp.pad(ssm_k, ((0, 0), (0, S)))
        kv_f = (lambda x, axes=(-2, -1): jnp.fft.rfft2(x.astype(jnp.float32), axes=axes))(kv_pad[:, None, :, :], axes=(1, 2))
        kf_f = (lambda x, axes=(-2, -1): jnp.fft.rfft2(x.astype(jnp.float32), axes=axes))(kf_pad[:, None, :], axes=(1, 2))
        kf_f = (lambda x, *d: x.transpose(*d))(kf_f, 1, 2, 0)
        y_f = kv_f * kf_f[None, :, :, :]
        y = (lambda x, s, axes=(-2, -1): jnp.fft.irfft2(x, s=s, axes=axes).astype(jnp.bfloat16))(y_f, (1, L), axes=(1, 2))[:, 0, :S, :]
        y = y + kv * ssm_D[None, None, :]
        return q * y

    def _B_ref(x, mem0, Wq, Wk, Wv, Wo, seg_len):
        B, S, Dm = x.shape
        H, Dh = (Wq.shape[1], Wq.shape[2])
        M = mem0.shape[1]
        scale = Dh ** (-0.5)
        n_seg = S // seg_len
        L = M + seg_len
        idx = jnp.arange(L)
        mask = (idx[:, None] < M) | (idx[:, None] >= idx[None, :])
        mem = mem0
        outs = []
        for s in range(n_seg):
            xs = x[:, s * seg_len:(s + 1) * seg_len, :].copy()
            h = jnp.concatenate([mem, xs], axis=1)
            q = jnp.einsum('btd,dhe->bhte', h, Wq)
            k = jnp.einsum('btd,dhe->bhte', h, Wk)
            v = jnp.einsum('btd,dhe->bhte', h, Wv)
            scores = jnp.einsum('bhqe,bhke->bhqk', q, k) * scale
            scores = jnp.where(mask[None, None], scores, -1000000000.0)
            p = _softmax(scores, axis=-1)
            o = jnp.einsum('bhqk,bhke->bhqe', p, v)
            o = jnp.einsum('bhte,hed->btd', o, Wo)
            mem = o[:, :M, :].copy()
            outs.append(o[:, M:, :])
        return jnp.concatenate(outs, axis=1)
    x = A_q
    g = _sigmoid((x * gate_w).sum(-1, keepdims=True))
    a = _A_ref(x, A_k, A_v, A_shift_k, A_ssm_k, A_ssm_D)
    b = _B_ref(x, B_mem0, B_Wq, B_Wk, B_Wv, B_Wo, B_seg_len)
    return g * a + (1 - g) * b
```

```python
import functools
import math

import numpy as np
import jax
import jax.numpy as jnp
import jax.experimental.pallas as pl
import jax.experimental.pallas.tpu as pltpu

F32 = jnp.float32
BF16 = jnp.bfloat16
U32 = jnp.uint32

def _add(a, b):
    return b if a is None else (a if b is None else a + b)
def _sub(a, b):
    return (None if b is None else -b) if a is None else (a if b is None else a - b)
def _cadd(a, b): return (_add(a[0], b[0]), _add(a[1], b[1]))
def _csub(a, b): return (_sub(a[0], b[0]), _sub(a[1], b[1]))
def _mulc(a, c):
    if a is None or abs(c) < 1e-12: return None
    if abs(c - 1) < 1e-12: return a
    if abs(c + 1) < 1e-12: return -a
    return a * np.float32(c)
def _ctw(z, num, den):
    num %= den
    re, im = z
    if (4 * num) % den == 0:
        qd = (4 * num) // den
        neg = lambda t: None if t is None else -t
        return [(re, im), (neg(im), re), (neg(re), neg(im)), (im, neg(re))][qd]
    c, s = math.cos(2 * math.pi * num / den), math.sin(2 * math.pi * num / den)
    if (8 * num) % den == 0 and re is not None and im is not None:
        sc, ss = (1 if c > 0 else -1), (1 if s > 0 else -1)
        r_ = re if sc > 0 else -re; i_ = im if sc > 0 else -im
        t = sc * ss
        a = (r_ - i_) if t > 0 else (r_ + i_)
        b = (i_ + r_) if t > 0 else (i_ - r_)
        return (a * np.float32(abs(c)), b * np.float32(abs(c)))
    return (_sub(_mulc(re, c), _mulc(im, s)), _add(_mulc(re, s), _mulc(im, c)))
def _cfft(zs, sign):
    n = len(zs)
    if n == 1: return list(zs)
    ev, od = _cfft(zs[0::2], sign), _cfft(zs[1::2], sign)
    out = [None] * n
    for j in range(n // 2):
        t = _ctw(od[j], sign * j, n)
        out[j] = _cadd(ev[j], t); out[j + n // 2] = _csub(ev[j], t)
    return out
def _conj(z): return (z[0], None if z[1] is None else -z[1])
def rfft_sym(xs):
    n = len(xs)
    if n == 1: return [(xs[0], None)]
    if n == 2: return [(_add(xs[0], xs[1]), None), (_sub(xs[0], xs[1]), None)]
    hf, q = n // 2, n // 4
    s = [_add(xs[i], xs[i + hf]) for i in range(hf)]
    d = [_sub(xs[i], xs[i + hf]) for i in range(hf)]
    out = [None] * (hf + 1)
    for j, e in enumerate(rfft_sym(s)): out[2 * j] = e
    z = [_ctw((d[i], None if d[i + q] is None else -d[i + q]), -i, n) for i in range(q)]
    for j, e in enumerate(_cfft(z, -1)):
        m = 4 * j + 1
        if m <= hf: out[m] = e
        else: out[n - m] = _conj(e)
    return out
def irfft_sym(U, n, nout):
    if n == 1: return [U[0][0]]
    if n == 2: return [_add(U[0][0], U[1][0]), _sub(U[0][0], U[1][0])][:nout]
    hf, q = n // 2, n // 4
    e = irfft_sym(U[0::2], hf, hf)
    V = []
    for j in range(q):
        m = 4 * j + 1
        V.append(U[m] if m <= hf else _conj(U[n - m]))
    w = _cfft(V, +1)
    o = [None] * hf
    for i in range(q):
        t = _ctw(w[i], i, n)
        o[i] = t[0]; o[i + q] = None if t[1] is None else -t[1]
    y = [_add(e[i], o[i]) for i in range(hf)]
    if nout > hf: y += [_sub(e[i], o[i]) for i in range(hf)]
    return y[:nout]


def _bf16_bits(a):
    u = np.ascontiguousarray(a, np.float32).view(np.uint32)
    return (u + 0x7FFF + ((u >> 16) & 1)) >> 16


def _pack_rows(a):
    b = _bf16_bits(a)
    return (b[0::2] | (b[1::2] << 16)).astype(np.uint32)


@functools.lru_cache(maxsize=None)
def _dft_tables(N1, N2, RI):
    Lf, hN = N1 * N2, N2 // 2
    k2 = np.arange(N2)[:, None]
    n2 = np.arange(N2)[None, :]
    perm = np.arange(2 * N2).reshape(2, N2 // RI, RI).transpose(1, 0, 2).reshape(-1)
    fw, inv = [], []
    for k1 in range(N1 // 2):
        f = np.zeros((2 * N2, 2 * N2))
        g = np.zeros((2 * N2, 2 * N2))
        if k1 > 0:
            ph = -2 * np.pi * ((k2 * n2 % N2) / N2 + (n2 * k1) / Lf)
            Fr, Fi = np.cos(ph), np.sin(ph)
            f[:N2, 0::2] = Fr; f[:N2, 1::2] = -Fi
            f[N2:, 0::2] = Fi; f[N2:, 1::2] = Fr
            Gr, Gi = Fr.T * (2.0 / Lf), -Fi.T * (2.0 / Lf)
            g[:N2, 0::2] = Gr; g[:N2, 1::2] = -Gi
            g[N2:, 0::2] = Gi; g[N2:, 1::2] = Gr
        else:
            kk = np.arange(hN)[:, None]
            p0 = -2 * np.pi * (kk * n2 % N2) / N2
            p1 = -2 * np.pi * ((kk * n2 % N2) / N2 + n2 * (N1 // 2) / Lf)
            F0r, F0i, F1r, F1i = np.cos(p0), np.sin(p0), np.cos(p1), np.sin(p1)
            nyq = np.cos(np.pi * n2[0])
            f[:hN, 0::2] = F0r; f[hN:N2, 1::2] = F1r
            f[N2:N2 + hN, 0::2] = F0i; f[N2 + hN:, 1::2] = F1i
            f[N2, 0::2] = nyq
            c = 2.0 / Lf
            g[:N2, 0:N2:2] = F0r.T * c; g[:N2, 1:N2:2] = F0i.T * c
            g[:N2, 0] = 1.0 / Lf; g[:N2, 1] = nyq / Lf
            g[N2:, N2::2] = F1r.T * c; g[N2:, N2 + 1::2] = F1i.T * c
        fw.append(_pack_rows(f[perm]))
        inv.append(_pack_rows(g))
    return np.stack(fw + inv)


CFG = dict(G=2, skew_s=1, skew_pv=3, skew_wo=2, WD=256, RI=16)


def _kernel(S, D, H, Dh, M, SEG, cfg,
            shift_ref, ssmD_ref, mem0_ref, gatew_ref,
            q_hbm, k_hbm, v_hbm, ssmk_hbm, wq_hbm, wk_hbm, wv_hbm, wo_hbm, tab_hbm,
            out_hbm,
            x_ref, k_ref, v_ref, ssm_ref, tab_ref, shT, kv_s, hT_s, A_s, Y_s, U_s, y_ref,
            wraw, wqkv, wo, h_ref, o_ref, acc_ref, out_ref, sems, osem):
    L = M + SEG
    n_seg = S // SEG
    HP = H // 2
    WD, RI = cfg["WD"], cfg["RI"]
    N2 = 128
    NB = S // N2
    NL = WD // 128
    NBLK = D // WD

    def cp_blk(b):
        ls = pl.ds(b * WD, WD)
        return [pltpu.make_async_copy(k_hbm.at[:, ls], k_ref.at[:, ls], sems.at[3 * b]),
                pltpu.make_async_copy(v_hbm.at[:, ls], v_ref.at[:, ls], sems.at[3 * b + 1]),
                pltpu.make_async_copy(ssmk_hbm.at[ls, :], ssm_ref.at[ls, :], sems.at[3 * b + 2])]

    def wraw_copy(src, slot, sem):
        return pltpu.make_async_copy(
            src.bitcast(U32).reshape(D * HP, Dh), wraw.at[slot], sems.at[sem])

    s0 = 3 * NBLK
    cp_tabF = pltpu.make_async_copy(tab_hbm.at[0:NB], tab_ref.at[0:NB], sems.at[s0])
    cp_tabG = pltpu.make_async_copy(tab_hbm.at[NB:], tab_ref.at[NB:], sems.at[s0 + 1])
    cp_w = [wraw_copy(w, i, s0 + 2 + i) for i, w in enumerate((wq_hbm, wk_hbm, wv_hbm))]
    cp_wo = pltpu.make_async_copy(wo_hbm.bitcast(U32), wo, sems.at[s0 + 5])
    X0 = 4 * SEG
    cp_x0 = pltpu.make_async_copy(q_hbm.at[0:X0], x_ref.at[0:X0], sems.at[s0 + 6])
    cp_x1 = pltpu.make_async_copy(q_hbm.at[X0:], x_ref.at[X0:], sems.at[s0 + 7])
    blk_cps = [cp_blk(b) for b in range(NBLK)]
    for b in range(NBLK):
        for c in blk_cps[b]:
            c.start()
        if b == 1:
            cp_tabF.start(); cp_tabG.start()
    for c in cp_w:
        c.start()
    cp_x0.start(); cp_wo.start(); cp_x1.start()

    shT[...] = jnp.concatenate(
        [shift_ref[...].astype(F32), jnp.zeros((D, 128 - shift_ref.shape[1]), F32)], axis=1).T[:8]
    ks_taps = shift_ref.shape[1]

    def st_kv(b, i):
        r0 = pl.multiple_of(i * N2, N2)
        rp = pl.multiple_of(jnp.maximum(r0 - 16, 0), 16)
        for j in range(NL):
            lg = pl.ds(b * WD + j * 128, 128)
            ll = pl.ds(j * 128, 128)
            cur = k_ref[pl.ds(r0, N2), lg].astype(F32)
            prev = jnp.where(i > 0, k_ref[pl.ds(rp, 16), lg].astype(F32), 0.0)
            ext = jnp.concatenate([prev[8:16], cur], axis=0)
            w = shT[:, lg]
            ks = cur * w[0:1]
            for t in range(1, ks_taps):
                ks = ks + ext[8 - t:8 - t + N2] * w[t:t + 1]
            kv = ks * v_ref[pl.ds(r0, N2), lg].astype(F32)
            kv_s[b % 2, pl.ds(r0, N2), ll] = kv
            y_ref[pl.ds(r0, N2), lg] = kv * ssmD_ref[:, lg].astype(F32)
            hT_s[b % 2, pl.ds(r0, N2), ll] = ssm_ref[lg, pl.ds(r0, N2)].astype(F32).T

    def st_a(b, i):
        r0 = pl.multiple_of(i * 8, 8)
        for src, off in ((kv_s, 0), (hT_s, WD)):
            for j in range(NL):
                xs = [src[b % 2, pl.ds(n1 * N2 + r0, 8), pl.ds(j * 128, 128)] for n1 in range(NB)]
                X = rfft_sym(xs + [None] * NB)
                for k1 in range(NB):
                    pair = [X[0][0], X[NB][0]] if k1 == 0 else [X[k1][0], X[k1][1]]
                    A_s[b % 2, k1, pl.ds(r0, 8), pl.ds(off + j * 128, 128)] = (
                        pltpu.pack_elementwise(pair, packed_dtype=BF16))

    def st_g1(b, i):
        Fm = pltpu.bitcast(tab_ref[i], BF16)
        Am = pltpu.bitcast(A_s[b % 2, i], BF16)
        X = jnp.dot(Fm, Am, preferred_element_type=F32)
        for r in range(N2 // RI):
            re = X[2 * r * RI:(2 * r + 1) * RI]
            im = X[(2 * r + 1) * RI:(2 * r + 2) * RI]
            a, c = re[:, :WD], re[:, WD:]
            b_, d = im[:, :WD], im[:, WD:]
            bd = b_ * d
            yre, yim = a * c - bd, a * d + b_ * c
            if r == 0:
                rid = jax.lax.broadcasted_iota(jnp.int32, (RI, WD), 0) + i
                yre = jnp.where(rid == 0, a * c, yre)
                yim = jnp.where(rid == 0, bd, yim)
            Y_s[i % 2, pl.ds(r * RI, RI), :] = pltpu.pack_elementwise([yre, yim], packed_dtype=BF16)

    def st_g2(b, i, ub):
        Gm = pltpu.bitcast(tab_ref[NB + i], BF16)
        Ym = pltpu.bitcast(Y_s[i % 2], BF16)
        U_s[ub, i] = jnp.dot(Gm, Ym, preferred_element_type=F32)

    def st_i(b, i):
        r0 = pl.multiple_of(i * 8, 8)
        for j in range(NL):
            lg = pl.ds(b * WD + j * 128, 128)
            ld = lambda k1, part: U_s[b % 2, k1, pl.ds(part * N2 + r0, 8), pl.ds(j * 128, 128)]
            U = [(ld(0, 0), None)] + [(ld(k1, 0), ld(k1, 1)) for k1 in range(1, NB)] + [(ld(0, 1), None)]
            ys = irfft_sym(U, 2 * NB, NB)
            for n1 in range(NB):
                rr = pl.ds(n1 * N2 + r0, 8)
                y_ref[rr, lg] = y_ref[rr, lg] + ys[n1]

    def st_relayout(slot, i, n_per):
        for u in range(n_per):
            ii = i * n_per + u
            r0 = pl.multiple_of(ii * 8, 8)
            for hp in range(HP):
                a = wraw[slot, pl.ds(ii * 16 * HP + hp, 8, stride=2 * HP), :]
                b = wraw[slot, pl.ds(ii * 16 * HP + HP + hp, 8, stride=2 * HP), :]
                c0 = (2 * hp) * 3 * Dh + slot * Dh
                wqkv[pl.ds(r0, 8), pl.ds(c0, Dh)] = (a & 0xFFFF) | (b << 16)
                wqkv[pl.ds(r0, 8), pl.ds(c0 + 3 * Dh, Dh)] = (a >> 16) | (b & np.uint32(0xFFFF0000))

    rel_slot = cfg.get("rel_slot", (NBLK, NBLK + 1, NBLK + 3))
    n_slots = max(NBLK + 3, max(rel_slot) + 1)
    for slot in range(n_slots):
        bk, ba, bg, bi = slot, slot - 1, slot - 2, slot - 3
        ok = lambda b: 0 <= b < NBLK
        if ok(bk):
            for c in blk_cps[bk]:
                c.wait()
        if bg == 0:
            cp_tabF.wait(); cp_tabG.wait()
        rel = [m for m in range(3) if rel_slot[m] == slot]
        for m in rel:
            cp_w[m].wait()

        def body(i, carry, bk=bk, ba=ba, bg=bg, bi=bi, rel=rel, first=False):
            if ok(bg):
                st_g1(bg, i)
                if not first:
                    st_g2(bg, i - 1, bg % 2)
            if ok(bi):
                st_i(bi, i)
            if ok(ba):
                st_a(ba, i)
            if ok(bk):
                st_kv(bk, i)
            for m in rel:
                st_relayout(m, i, D // 16 // NB)
            return carry

        if ok(bg):
            body(0, 0, first=True)
            jax.lax.fori_loop(1, NB, body, 0)
            st_g2(bg, NB - 1, bg % 2)
        else:
            jax.lax.fori_loop(0, NB, body, 0)

    cp_x0.wait()
    cp_wo.wait()

    scale = Dh ** (-0.5)
    G = cfg["G"]
    gate_w = gatew_ref[...].astype(F32)

    def step(s, mem):
        r0 = pl.multiple_of(s * SEG, SEG)
        xs = x_ref[pl.ds(r0, SEG), :].astype(F32)
        h_ref[0:M, :] = mem
        h_ref[M:L, :] = xs
        row = jax.lax.broadcasted_iota(jnp.int32, (L, L), 0)
        col = jax.lax.broadcasted_iota(jnp.int32, (L, L), 1)
        mask = (row < M) | (row >= col)

        qkv = {}
        probs = {}

        def proj(h):
            w = pltpu.bitcast(wqkv[:, pl.ds(h * 3 * Dh, 3 * Dh)], BF16)
            r = jax.lax.dot_general(h_ref[...], w, (((1,), (0,)), ((), ())),
                                    preferred_element_type=F32)
            qkv[h] = (r[:, :Dh].astype(BF16), r[:, Dh:2 * Dh].astype(BF16), r[:, 2 * Dh:].astype(BF16))

        def scores(h):
            q, k, _ = qkv[h]
            sc = jax.lax.dot_general(q, k, (((1,), (1,)), ((), ())),
                                     preferred_element_type=F32) * scale
            sc = jnp.where(mask, sc, -1e9)
            m = jnp.max(sc, axis=-1, keepdims=True)
            e = jnp.exp(sc - m)
            probs[h] = (e / jnp.sum(e, axis=-1, keepdims=True)).astype(BF16)

        def pv(h):
            o = jnp.dot(probs.pop(h), qkv.pop(h)[2], preferred_element_type=F32)
            o_ref[:, pl.ds(h * Dh, Dh)] = o

        def wo_group(g):
            w = pltpu.bitcast(wo[pl.ds(g * G * Dh // 2, G * Dh // 2), :], BF16)
            r = jax.lax.dot_general(o_ref[:, pl.ds(g * G * Dh, G * Dh)], w,
                                    (((1,), (0,)), ((), ())), preferred_element_type=F32)
            if g == 0:
                acc_ref[...] = r
            elif g < H // G - 1:
                acc_ref[...] += r
            else:
                return acc_ref[...] + r

        s1, s2, s3 = cfg["skew_s"], cfg["skew_pv"], cfg["skew_wo"]
        res = None
        for t in range(H + s1 + s2 + s3):
            if t < H:
                proj(t)
            if 0 <= t - s1 < H:
                scores(t - s1)
            hh = t - s1 - s2
            if 0 <= hh < H:
                pv(hh)
            hw = t - s1 - s2 - s3
            if 0 <= hw < H and (hw + 1) % G == 0:
                res = wo_group(hw // G)
        mem_next = res[0:M, :].astype(BF16).astype(F32)
        b = res[M:L, :]
        g = jax.nn.sigmoid(jnp.sum(xs * gate_w, axis=-1, keepdims=True))
        a = xs * y_ref[pl.ds(r0, SEG), :]
        out_ref[pl.ds(r0, SEG), :] = (g * a + (1.0 - g) * b).astype(out_ref.dtype)
        pltpu.make_async_copy(out_ref.at[pl.ds(r0, SEG)], out_hbm.at[pl.ds(r0, SEG)], osem).start()
        return mem_next

    nst = cfg.get("nsteps", n_seg)
    n1 = X0 // SEG
    mem = jax.lax.fori_loop(0, n1, step, mem0_ref[...].astype(F32))
    cp_x1.wait()
    jax.lax.fori_loop(n1, nst, step, mem)
    pltpu.make_async_copy(out_ref.at[0:nst * SEG], out_hbm.at[0:nst * SEG], osem).wait()


@functools.partial(jax.jit, static_argnames=("B_seg_len", "cfg"))
def pallas_gated_mix__ssm_conv_h3__memory_aug_recurrent_mem_tr__prompt_kernel(
    A_q, A_k, A_v, A_shift_k, A_ssm_k, A_ssm_D, B_x, B_mem0, B_Wq, B_Wk, B_Wv, B_Wo,
    B_seg_len, gate_w, cfg=None,
):
    del B_x
    cfg = dict(CFG, **dict(cfg or ()))
    _, S, D = A_q.shape
    _, H, Dh = B_Wq.shape
    M = B_mem0.shape[1]
    SEG = int(B_seg_len)
    L = M + SEG
    WD = cfg["WD"]
    NB = S // 128
    tab = _dft_tables(2 * NB, 128, cfg["RI"])
    kern = functools.partial(_kernel, S, D, H, Dh, M, SEG, cfg)
    vm = pl.BlockSpec(memory_space=pltpu.VMEM)
    hbm = pl.BlockSpec(memory_space=pl.ANY)
    out = pl.pallas_call(
        kern,
        out_shape=jax.ShapeDtypeStruct((S, D), BF16),
        in_specs=[vm, vm, vm, vm] + [hbm] * 9,
        out_specs=hbm,
        scratch_shapes=[
            pltpu.VMEM((S, D), BF16),
            pltpu.VMEM((S, D), BF16),
            pltpu.VMEM((S, D), BF16),
            pltpu.VMEM((D, S), BF16),
            pltpu.VMEM(tab.shape, U32),
            pltpu.VMEM((8, D), F32),
            pltpu.VMEM((2, S, WD), F32),
            pltpu.VMEM((2, S, WD), F32),
            pltpu.VMEM((2, NB, 128, 2 * WD), U32),
            pltpu.VMEM((2, 128, WD), U32),
            pltpu.VMEM((2, NB, 256, WD), F32),
            pltpu.VMEM((S, D), F32),
            pltpu.VMEM((3, D * H // 2, Dh), U32),
            pltpu.VMEM((D // 2, 3 * H * Dh), U32),
            pltpu.VMEM((H * Dh // 2, D), U32),
            pltpu.VMEM((L, D), F32),
            pltpu.VMEM((L, H * Dh), F32),
            pltpu.VMEM((L, D), F32),
            pltpu.VMEM((S, D), BF16),
            pltpu.SemaphoreType.DMA((3 * (D // WD) + 8,)),
            pltpu.SemaphoreType.DMA,
        ],
        compiler_params=pltpu.CompilerParams(vmem_limit_bytes=120 * 1024 * 1024),
    )(
        A_shift_k, A_ssm_D.reshape(1, D), B_mem0.reshape(M, D), gate_w.reshape(1, D),
        A_q.reshape(S, D), A_k.reshape(S, D), A_v.reshape(S, D), A_ssm_k,
        B_Wq, B_Wk, B_Wv, B_Wo.reshape(H * Dh, D), tab,
    )
    return out.reshape(1, S, D)
```

```python
import functools
import math

import numpy as np
import jax
import jax.numpy as jnp
import jax.experimental.pallas as pl
import jax.experimental.pallas.tpu as pltpu

F32 = jnp.float32
BF16 = jnp.bfloat16
U32 = jnp.uint32

def _add(a, b):
    return b if a is None else (a if b is None else a + b)
def _sub(a, b):
    return (None if b is None else -b) if a is None else (a if b is None else a - b)
def _cadd(a, b): return (_add(a[0], b[0]), _add(a[1], b[1]))
def _csub(a, b): return (_sub(a[0], b[0]), _sub(a[1], b[1]))
def _mulc(a, c):
    if a is None or abs(c) < 1e-12: return None
    if abs(c - 1) < 1e-12: return a
    if abs(c + 1) < 1e-12: return -a
    return a * np.float32(c)
def _ctw(z, num, den):
    num %= den
    re, im = z
    if (4 * num) % den == 0:
        qd = (4 * num) // den
        neg = lambda t: None if t is None else -t
        return [(re, im), (neg(im), re), (neg(re), neg(im)), (im, neg(re))][qd]
    c, s = math.cos(2 * math.pi * num / den), math.sin(2 * math.pi * num / den)
    if (8 * num) % den == 0 and re is not None and im is not None:
        sc, ss = (1 if c > 0 else -1), (1 if s > 0 else -1)
        r_ = re if sc > 0 else -re; i_ = im if sc > 0 else -im
        t = sc * ss
        a = (r_ - i_) if t > 0 else (r_ + i_)
        b = (i_ + r_) if t > 0 else (i_ - r_)
        return (a * np.float32(abs(c)), b * np.float32(abs(c)))
    return (_sub(_mulc(re, c), _mulc(im, s)), _add(_mulc(re, s), _mulc(im, c)))
def _cfft(zs, sign):
    n = len(zs)
    if n == 1: return list(zs)
    ev, od = _cfft(zs[0::2], sign), _cfft(zs[1::2], sign)
    out = [None] * n
    for j in range(n // 2):
        t = _ctw(od[j], sign * j, n)
        out[j] = _cadd(ev[j], t); out[j + n // 2] = _csub(ev[j], t)
    return out
def _conj(z): return (z[0], None if z[1] is None else -z[1])
def rfft_sym(xs):
    n = len(xs)
    if n == 1: return [(xs[0], None)]
    if n == 2: return [(_add(xs[0], xs[1]), None), (_sub(xs[0], xs[1]), None)]
    hf, q = n // 2, n // 4
    s = [_add(xs[i], xs[i + hf]) for i in range(hf)]
    d = [_sub(xs[i], xs[i + hf]) for i in range(hf)]
    out = [None] * (hf + 1)
    for j, e in enumerate(rfft_sym(s)): out[2 * j] = e
    z = [_ctw((d[i], None if d[i + q] is None else -d[i + q]), -i, n) for i in range(q)]
    for j, e in enumerate(_cfft(z, -1)):
        m = 4 * j + 1
        if m <= hf: out[m] = e
        else: out[n - m] = _conj(e)
    return out
def irfft_sym(U, n, nout):
    if n == 1: return [U[0][0]]
    if n == 2: return [_add(U[0][0], U[1][0]), _sub(U[0][0], U[1][0])][:nout]
    hf, q = n // 2, n // 4
    e = irfft_sym(U[0::2], hf, hf)
    V = []
    for j in range(q):
        m = 4 * j + 1
        V.append(U[m] if m <= hf else _conj(U[n - m]))
    w = _cfft(V, +1)
    o = [None] * hf
    for i in range(q):
        t = _ctw(w[i], i, n)
        o[i] = t[0]; o[i + q] = None if t[1] is None else -t[1]
    y = [_add(e[i], o[i]) for i in range(hf)]
    if nout > hf: y += [_sub(e[i], o[i]) for i in range(hf)]
    return y[:nout]


def _bf16_bits(a):
    u = np.ascontiguousarray(a, np.float32).view(np.uint32)
    return (u + 0x7FFF + ((u >> 16) & 1)) >> 16


def _pack_rows(a):
    b = _bf16_bits(a)
    r = b.shape[0] // 2
    return (b[:r] | (b[r:] << 16)).astype(np.uint32)


@functools.lru_cache(maxsize=None)
def _dft_consts(N1, N2, RI):
    Lf, hN = N1 * N2, N2 // 2
    k2 = np.arange(N2)[:, None]
    n2 = np.arange(N2)[None, :]
    ph = -2 * np.pi * (k2 * n2 % N2) / N2
    Fr, Fi = np.cos(ph), np.sin(ph)
    Gr, Gi = Fr.T * (2.0 / Lf), -Fi.T * (2.0 / Lf)

    def inter(a, b):
        m = np.zeros((N2, 2 * N2))
        m[:, 0::2] = a; m[:, 1::2] = b
        return m
    base = np.stack([inter(Fr, -Fi), inter(Fi, Fr), inter(Gr, -Gi), inter(Gi, Gr)]).astype(np.float32)
    th = 2 * np.pi * np.arange(N1 // 2)[:, None] * np.arange(N2)[None, :] / Lf
    twf = np.stack([np.repeat(np.cos(th), 2, axis=1), np.repeat(np.sin(th), 2, axis=1)]).astype(np.float32)
    twg = np.zeros((N2, 128), np.float32)
    twg[:, :N1 // 2] = np.cos(th).T; twg[:, 64:64 + N1 // 2] = np.sin(th).T
    f = np.zeros((2 * N2, 2 * N2))
    g = np.zeros((2 * N2, 2 * N2))
    kk = np.arange(hN)[:, None]
    p0 = -2 * np.pi * (kk * n2 % N2) / N2
    p1 = -2 * np.pi * ((kk * n2 % N2) / N2 + n2 * (N1 // 2) / Lf)
    F0r, F0i, F1r, F1i = np.cos(p0), np.sin(p0), np.cos(p1), np.sin(p1)
    nyq = np.cos(np.pi * n2[0])
    f[:hN, 0::2] = F0r; f[hN:N2, 1::2] = F1r
    f[N2:N2 + hN, 0::2] = F0i; f[N2 + hN:, 1::2] = F1i
    f[N2, 0::2] = nyq
    c = 2.0 / Lf
    g[:N2, 0:N2:2] = F0r.T * c; g[:N2, 1:N2:2] = F0i.T * c
    g[:N2, 0] = 1.0 / Lf; g[:N2, 1] = nyq / Lf
    g[N2:, N2::2] = F1r.T * c; g[N2:, N2 + 1::2] = F1i.T * c
    perm = np.arange(2 * N2).reshape(2, N2 // RI, RI).transpose(1, 0, 2).reshape(-1)
    sp = np.stack([_pack_rows(f[perm]), _pack_rows(g)])
    return base, twf, twg, sp


CFG = dict(G=2, skew_s=1, skew_pv=5, skew_wo=4, WD=256, RI=8, MS=128, MS2=128, hT="mxu", order="21IAKR", unroll=1)


def _kernel(S, D, H, Dh, M, SEG, cfg,
            shift_ref, ssmD_ref, mem0_ref, gatew_ref,
            q_hbm, k_hbm, v_hbm, ssmk_hbm, wq_hbm, wk_hbm, wv_hbm, wo_hbm, cb_hbm, ctf_hbm, ctg_hbm, csp_hbm,
            out_hbm,
            x_ref, k_ref, v_ref, ssm_ref, tab_ref, cb_ref, ctf_ref, ctg_ref, shT, kv_s, hT_s, A_s, Y_s, U_s, y_ref,
            wraw, wqkv, wo, h_ref, o_ref, acc_ref, out_ref, sems, osem):
    L = M + SEG
    n_seg = S // SEG
    HP = H // 2
    WD, RI = cfg["WD"], cfg["RI"]
    N2 = 128
    NB = S // N2
    NL = WD // 128
    NBLK = D // WD

    def cp_blk(b):
        ls = pl.ds(b * WD, WD)
        return [pltpu.make_async_copy(k_hbm.at[:, ls], k_ref.at[:, ls], sems.at[3 * b]),
                pltpu.make_async_copy(v_hbm.at[:, ls], v_ref.at[:, ls], sems.at[3 * b + 1]),
                pltpu.make_async_copy(ssmk_hbm.at[ls, :], ssm_ref.at[ls, :], sems.at[3 * b + 2])]

    def wraw_copy(src, slot, sem):
        return pltpu.make_async_copy(
            src.bitcast(U32).reshape(D * HP, Dh), wraw.at[slot], sems.at[sem])

    s0 = 3 * NBLK
    cp_c = [pltpu.make_async_copy(cb_hbm, cb_ref, sems.at[s0]),
            pltpu.make_async_copy(ctf_hbm, ctf_ref, sems.at[s0 + 1]),
            pltpu.make_async_copy(ctg_hbm, ctg_ref, sems.at[s0 + 8]),
            pltpu.make_async_copy(csp_hbm.at[0], tab_ref.at[0], sems.at[s0 + 9]),
            pltpu.make_async_copy(csp_hbm.at[1], tab_ref.at[NB], sems.at[s0 + 10])]
    cp_w = [wraw_copy(w, i, s0 + 2 + i) for i, w in enumerate((wq_hbm, wk_hbm, wv_hbm))]
    cp_wo = pltpu.make_async_copy(wo_hbm.bitcast(U32), wo, sems.at[s0 + 5])
    X0 = 4 * SEG
    cp_x0 = pltpu.make_async_copy(q_hbm.at[0:X0], x_ref.at[0:X0], sems.at[s0 + 6])
    cp_x1 = pltpu.make_async_copy(q_hbm.at[X0:], x_ref.at[X0:], sems.at[s0 + 7])
    blk_cps = [cp_blk(b) for b in range(NBLK)]
    for c in cp_c:
        c.start()
    for b in range(NBLK):
        for c in blk_cps[b]:
            c.start()
    late = cp_w + [cp_x0, cp_wo, cp_x1]
    w_start = cfg.get("w_start", (0, 0, 0, 0, 0, 0))
    for c, sl in zip(late, w_start):
        if sl == 0:
            c.start()

    shT[...] = jnp.concatenate(
        [shift_ref[...].astype(F32), jnp.zeros((D, 128 - shift_ref.shape[1]), F32)], axis=1).T[:8]
    ks_taps = shift_ref.shape[1]
    eye = (jax.lax.broadcasted_iota(jnp.int32, (N2, N2), 0)
           == jax.lax.broadcasted_iota(jnp.int32, (N2, N2), 1)).astype(BF16)

    for c in cp_c:
        c.wait()
    hq = N2 // 2
    for k1 in range(1, NB):
        cf, sf = ctf_ref[0, k1:k1 + 1, :], ctf_ref[1, k1:k1 + 1, :]
        for q in range(N2 // 8):
            g8 = (q // 2) * 8

            def rot(r):
                fre, fim = cb_ref[0, r:r + 8, :], cb_ref[1, r:r + 8, :]
                return fre * cf + fim * sf if q % 2 == 0 else fim * cf - fre * sf
            tab_ref[k1, q * 8:q * 8 + 8, :] = pltpu.pack_elementwise([rot(g8), rot(hq + g8)], packed_dtype=BF16)
            rows = slice(q * 8, q * 8 + 8)
            cg = jnp.broadcast_to(ctg_ref[rows, k1:k1 + 1], (8, 2 * N2))
            sg = jnp.broadcast_to(ctg_ref[rows, 64 + k1:64 + k1 + 1], (8, 2 * N2))
            gre, gim = cb_ref[2, rows, :], cb_ref[3, rows, :]
            tab_ref[NB + k1, rows, :] = pltpu.pack_elementwise(
                [gre * cg - gim * sg, gim * cg + gre * sg], packed_dtype=BF16)

    def st_kv(b, i):
        r0 = pl.multiple_of(i * N2, N2)
        rp = pl.multiple_of(jnp.maximum(r0 - 16, 0), 16)
        for j in range(NL):
            lg = pl.ds(b * WD + j * 128, 128)
            ll = pl.ds(j * 128, 128)
            cur = k_ref[pl.ds(r0, N2), lg].astype(F32)
            prev = jnp.where(i > 0, k_ref[pl.ds(rp, 16), lg].astype(F32), 0.0)
            ext = jnp.concatenate([prev[8:16], cur], axis=0)
            w = shT[:, lg]
            ks = cur * w[0:1]
            for t in range(1, ks_taps):
                ks = ks + ext[8 - t:8 - t + N2] * w[t:t + 1]
            kv = ks * v_ref[pl.ds(r0, N2), lg].astype(F32)
            kv_s[b % 2, pl.ds(r0, N2), ll] = kv
            y_ref[pl.ds(r0, N2), lg] = kv * ssmD_ref[:, lg].astype(F32)
            if cfg["hT"] == "xlu":
                hT_s[b % 2, pl.ds(r0, N2), ll] = ssm_ref[lg, pl.ds(r0, N2)].astype(F32).T
            else:
                hT_s[b % 2, pl.ds(r0, N2), ll] = jax.lax.dot_general(
                    eye, ssm_ref[lg, pl.ds(r0, N2)], (((1,), (1,)), ((), ())), preferred_element_type=F32)

    def st_a(b, i):
        r0 = pl.multiple_of(i * 8, 8)
        for src, off in ((kv_s, 0), (hT_s, 128)):
            for j in range(NL):
                xs = [src[b % 2, pl.ds(n1 * N2 + r0, 8), pl.ds(j * 128, 128)] for n1 in range(NB)]
                X = rfft_sym(xs + [None] * NB)
                for k1 in range(NB):
                    pair = [X[0][0], X[NB][0]] if k1 == 0 else [X[k1][0], X[k1][1]]
                    A_s[b % 2, k1, pl.ds(r0, 8), pl.ds(off + j * 256, 128)] = (
                        pltpu.pack_elementwise(pair, packed_dtype=BF16))

    def table(idx):
        w = tab_ref[idx]
        return jnp.concatenate([pltpu.bitcast(w << 16, F32),
                                pltpu.bitcast(w & np.uint32(0xFFFF0000), F32)], axis=0)

    def mm(a, b):
        return jax.lax.dot_general(a, b, (((1,), (0,)), ((), ())), preferred_element_type=F32)

    def st_g1(b, i, par):
        Fm = table(i)
        MS = cfg["MS"]
        for j in range(NL):
            Am = pltpu.bitcast(A_s[b % 2, i, :, pl.ds(j * 256, 256)], BF16)
            for m0 in range(0, 2 * N2, MS):
                X = mm(Fm[m0:m0 + MS], Am)
                for r in range(MS // (2 * RI)):
                    re = X[2 * r * RI:(2 * r + 1) * RI]
                    im = X[(2 * r + 1) * RI:(2 * r + 2) * RI]
                    a, c = re[:, :128], re[:, 128:]
                    b_, d = im[:, :128], im[:, 128:]
                    bd = b_ * d
                    yre, yim = a * c - bd, a * d + b_ * c
                    row = m0 // 2 + r * RI
                    if row == 0:
                        rid = jax.lax.broadcasted_iota(jnp.int32, (RI, 128), 0) + i
                        yre = jnp.where(rid == 0, a * c, yre)
                        yim = jnp.where(rid == 0, bd, yim)
                    Y_s[par, pl.ds(row, RI), pl.ds(j * 128, 128)] = (
                        pltpu.pack_elementwise([yre, yim], packed_dtype=BF16))

    def st_g2(b, i, par):
        Gm = table(NB + i)
        MS = cfg["MS2"]
        Ym = pltpu.bitcast(Y_s[par], BF16)
        for m0 in range(0, 2 * N2, MS):
            U_s[b % 2, i, pl.ds(m0, MS), :] = mm(Gm[m0:m0 + MS], Ym)

    def st_i(b, i):
        r0 = pl.multiple_of(i * 8, 8)
        for j in range(NL):
            lg = pl.ds(b * WD + j * 128, 128)
            ld = lambda k1, part: U_s[b % 2, k1, pl.ds(part * N2 + r0, 8), pl.ds(j * 128, 128)]
            U = [(ld(0, 0), None)] + [(ld(k1, 0), ld(k1, 1)) for k1 in range(1, NB)] + [(ld(0, 1), None)]
            ys = irfft_sym(U, 2 * NB, NB)
            for n1 in range(NB):
                rr = pl.ds(n1 * N2 + r0, 8)
                y_ref[rr, lg] = y_ref[rr, lg] + ys[n1]

    def st_relayout(slot, i, n_per):
        for u in range(n_per):
            ii = i * n_per + u
            r0 = pl.multiple_of(ii * 8, 8)
            for hp in range(HP):
                a = wraw[slot, pl.ds(ii * 16 * HP + hp, 8, stride=2 * HP), :]
                b = wraw[slot, pl.ds(ii * 16 * HP + HP + hp, 8, stride=2 * HP), :]
                c0 = (2 * hp) * 3 * Dh + slot * Dh
                wqkv[pl.ds(r0, 8), pl.ds(c0, Dh)] = (a & 0xFFFF) | (b << 16)
                wqkv[pl.ds(r0, 8), pl.ds(c0 + 3 * Dh, Dh)] = (a >> 16) | (b & np.uint32(0xFFFF0000))

    rel_slot = cfg.get("rel_slot", (NBLK - 1, NBLK, NBLK + 1))
    n_slots = max(NBLK + 3, max(rel_slot) + 1)
    for slot in range(n_slots):
        bk, ba, bg, bi = slot, slot - 1, slot - 2, slot - 3
        ok = lambda b: 0 <= b < NBLK
        sc_ = jax.named_scope(f"wait{slot}"); sc_.__enter__()
        if ok(bk):
            for c in blk_cps[bk]:
                c.wait()
        for c, sl in zip(late, w_start):
            if sl == slot and sl > 0:
                c.start()
        rel = [m for m in range(3) if rel_slot[m] == slot]
        for m in rel:
            cp_w[m].wait()
        sc_.__exit__(None, None, None)
        sc_ = jax.named_scope(f"slot{slot}"); sc_.__enter__()

        def body1(i, par, first=False, bk=bk, ba=ba, bg=bg, bi=bi, rel=rel):
            for st in cfg["order"]:
                if st == "1" and ok(bg):
                    st_g1(bg, i, par)
                elif st == "2" and ok(bg) and not first:
                    st_g2(bg, i - 1, 1 - par)
                elif st == "I" and ok(bi):
                    st_i(bi, i)
                elif st == "A" and ok(ba):
                    st_a(ba, i)
                elif st == "K" and ok(bk):
                    st_kv(bk, i)
                elif st == "R":
                    for m in rel:
                        st_relayout(m, i, D // 16 // NB)

        UN = cfg["unroll"]

        def body(i0, carry):
            for u in range(UN):
                body1(i0 * UN + u, u % 2 if UN > 1 else (i0 % 2))
            return carry

        if ok(bg):
            for u in range(UN):
                body1(u, u % 2, first=(u == 0))
            jax.lax.fori_loop(1, NB // UN, body, 0)
            st_g2(bg, NB - 1, (NB - 1) % 2)
        else:
            jax.lax.fori_loop(0, NB // UN, body, 0)
        sc_.__exit__(None, None, None)

    cp_x0.wait()
    cp_wo.wait()

    scale = Dh ** (-0.5)
    G = cfg["G"]
    gate_w = gatew_ref[...].astype(F32)

    def step(s, mem):
        r0 = pl.multiple_of(s * SEG, SEG)
        xs = x_ref[pl.ds(r0, SEG), :].astype(F32)
        h_ref[0:M, :] = mem
        h_ref[M:L, :] = xs
        row = jax.lax.broadcasted_iota(jnp.int32, (L, L), 0)
        col = jax.lax.broadcasted_iota(jnp.int32, (L, L), 1)
        mask = (row < M) | (row >= col)

        qkv = {}
        probs = {}

        def proj(h):
            w = pltpu.bitcast(wqkv[:, pl.ds(h * 3 * Dh, 3 * Dh)], BF16)
            r = jax.lax.dot_general(h_ref[...], w, (((1,), (0,)), ((), ())),
                                    preferred_element_type=F32)
            qkv[h] = (r[:, :Dh], r[:, Dh:2 * Dh].astype(BF16), r[:, 2 * Dh:].astype(BF16))

        def scores(h):
            q, k, _ = qkv[h]
            sc = jax.lax.dot_general(q, k, (((1,), (1,)), ((), ())),
                                     preferred_element_type=F32) * scale
            sc = jnp.where(mask, sc, -1e9)
            m = jnp.max(sc, axis=-1, keepdims=True)
            e = jnp.exp(sc - m)
            probs[h] = e / jnp.sum(e, axis=-1, keepdims=True)

        def pv(h):
            o = jnp.dot(probs.pop(h), qkv.pop(h)[2], preferred_element_type=F32)
            o_ref[:, pl.ds(h * Dh, Dh)] = o

        def wo_group(g):
            w = pltpu.bitcast(wo[pl.ds(g * G * Dh // 2, G * Dh // 2), :], BF16)
            r = jax.lax.dot_general(o_ref[:, pl.ds(g * G * Dh, G * Dh)], w,
                                    (((1,), (0,)), ((), ())), preferred_element_type=F32)
            if g == 0:
                acc_ref[...] = r
            elif g < H // G - 1:
                acc_ref[...] += r
            else:
                return acc_ref[...] + r

        s1, s2, s3 = cfg["skew_s"], cfg["skew_pv"], cfg["skew_wo"]
        res = None
        for t in range(H + s1 + s2 + s3):
            if t < H:
                proj(t)
            if 0 <= t - s1 < H:
                scores(t - s1)
            hh = t - s1 - s2
            if 0 <= hh < H:
                pv(hh)
            hw = t - s1 - s2 - s3
            if 0 <= hw < H and (hw + 1) % G == 0:
                res = wo_group(hw // G)
        mem_next = res[0:M, :].astype(BF16).astype(F32)
        b = res[M:L, :]
        g = jax.nn.sigmoid(jnp.sum(xs * gate_w, axis=-1, keepdims=True))
        a = xs * y_ref[pl.ds(r0, SEG), :]
        out_ref[pl.ds(r0, SEG), :] = (g * a + (1.0 - g) * b).astype(out_ref.dtype)
        pltpu.make_async_copy(out_ref.at[pl.ds(r0, SEG)], out_hbm.at[pl.ds(r0, SEG)], osem).start()
        return mem_next

    nst = cfg.get("nsteps", n_seg)
    n1 = X0 // SEG
    mem = jax.lax.fori_loop(0, n1, step, mem0_ref[...].astype(F32))
    cp_x1.wait()
    jax.lax.fori_loop(n1, nst, step, mem)
    pltpu.make_async_copy(out_ref.at[0:nst * SEG], out_hbm.at[0:nst * SEG], osem).wait()


@functools.partial(jax.jit, static_argnames=("B_seg_len", "cfg"))
def pallas_gated_mix__ssm_conv_h3__memory_aug_recurrent_mem_tr__prompt_kernel(
    A_q, A_k, A_v, A_shift_k, A_ssm_k, A_ssm_D, B_x, B_mem0, B_Wq, B_Wk, B_Wv, B_Wo,
    B_seg_len, gate_w, cfg=None,
):
    del B_x
    cfg = dict(CFG, **dict(cfg or ()))
    _, S, D = A_q.shape
    _, H, Dh = B_Wq.shape
    M = B_mem0.shape[1]
    SEG = int(B_seg_len)
    L = M + SEG
    WD = cfg["WD"]
    NB = S // 128
    assert cfg["RI"] == 8
    consts = _dft_consts(2 * NB, 128, cfg["RI"])
    kern = functools.partial(_kernel, S, D, H, Dh, M, SEG, cfg)
    vm = pl.BlockSpec(memory_space=pltpu.VMEM)
    hbm = pl.BlockSpec(memory_space=pl.ANY)
    out = pl.pallas_call(
        kern,
        out_shape=jax.ShapeDtypeStruct((S, D), BF16),
        in_specs=[vm, vm, vm, vm] + [hbm] * 12,
        out_specs=hbm,
        scratch_shapes=[
            pltpu.VMEM((S, D), BF16),
            pltpu.VMEM((S, D), BF16),
            pltpu.VMEM((S, D), BF16),
            pltpu.VMEM((D, S), BF16),
            pltpu.VMEM((2 * NB, 128, 256), U32),
            pltpu.VMEM(consts[0].shape, F32),
            pltpu.VMEM(consts[1].shape, F32),
            pltpu.VMEM(consts[2].shape, F32),
            pltpu.VMEM((8, D), F32),
            pltpu.VMEM((2, S, WD), F32),
            pltpu.VMEM((2, S, WD), F32),
            pltpu.VMEM((2, NB, 128, 2 * WD), U32),
            pltpu.VMEM((2, 128, WD), U32),
            pltpu.VMEM((2, NB, 256, WD), F32),
            pltpu.VMEM((S, D), F32),
            pltpu.VMEM((3, D * H // 2, Dh), U32),
            pltpu.VMEM((D // 2, 3 * H * Dh), U32),
            pltpu.VMEM((H * Dh // 2, D), U32),
            pltpu.VMEM((L, D), F32),
            pltpu.VMEM((L, H * Dh), F32),
            pltpu.VMEM((L, D), F32),
            pltpu.VMEM((S, D), BF16),
            pltpu.SemaphoreType.DMA((3 * (D // WD) + 11,)),
            pltpu.SemaphoreType.DMA,
        ],
        compiler_params=pltpu.CompilerParams(vmem_limit_bytes=120 * 1024 * 1024),
    )(
        A_shift_k, A_ssm_D.reshape(1, D), B_mem0.reshape(M, D), gate_w.reshape(1, D),
        A_q.reshape(S, D), A_k.reshape(S, D), A_v.reshape(S, D), A_ssm_k,
        B_Wq, B_Wk, B_Wv, B_Wo.reshape(H * Dh, D), *consts,
    )
    return out.reshape(1, S, D)
```

```python
import contextlib
import functools
import math

import numpy as np
import jax
import jax.numpy as jnp
import jax.experimental.pallas as pl
import jax.experimental.pallas.tpu as pltpu

F32 = jnp.float32
BF16 = jnp.bfloat16
U32 = jnp.uint32

def _add(a, b):
    return b if a is None else (a if b is None else a + b)
def _sub(a, b):
    return (None if b is None else -b) if a is None else (a if b is None else a - b)
def _cadd(a, b): return (_add(a[0], b[0]), _add(a[1], b[1]))
def _csub(a, b): return (_sub(a[0], b[0]), _sub(a[1], b[1]))
def _mulc(a, c):
    if a is None or abs(c) < 1e-12: return None
    if abs(c - 1) < 1e-12: return a
    if abs(c + 1) < 1e-12: return -a
    return a * np.float32(c)
def _ctw(z, num, den):
    num %= den
    re, im = z
    if (4 * num) % den == 0:
        qd = (4 * num) // den
        neg = lambda t: None if t is None else -t
        return [(re, im), (neg(im), re), (neg(re), neg(im)), (im, neg(re))][qd]
    c, s = math.cos(2 * math.pi * num / den), math.sin(2 * math.pi * num / den)
    if (8 * num) % den == 0 and re is not None and im is not None:
        sc, ss = (1 if c > 0 else -1), (1 if s > 0 else -1)
        r_ = re if sc > 0 else -re; i_ = im if sc > 0 else -im
        t = sc * ss
        a = (r_ - i_) if t > 0 else (r_ + i_)
        b = (i_ + r_) if t > 0 else (i_ - r_)
        return (a * np.float32(abs(c)), b * np.float32(abs(c)))
    return (_sub(_mulc(re, c), _mulc(im, s)), _add(_mulc(re, s), _mulc(im, c)))
def _cfft(zs, sign):
    n = len(zs)
    if n == 1: return list(zs)
    ev, od = _cfft(zs[0::2], sign), _cfft(zs[1::2], sign)
    out = [None] * n
    for j in range(n // 2):
        t = _ctw(od[j], sign * j, n)
        out[j] = _cadd(ev[j], t); out[j + n // 2] = _csub(ev[j], t)
    return out
def _conj(z): return (z[0], None if z[1] is None else -z[1])
def rfft_sym(xs):
    n = len(xs)
    if n == 1: return [(xs[0], None)]
    if n == 2: return [(_add(xs[0], xs[1]), None), (_sub(xs[0], xs[1]), None)]
    hf, q = n // 2, n // 4
    s = [_add(xs[i], xs[i + hf]) for i in range(hf)]
    d = [_sub(xs[i], xs[i + hf]) for i in range(hf)]
    out = [None] * (hf + 1)
    for j, e in enumerate(rfft_sym(s)): out[2 * j] = e
    z = [_ctw((d[i], None if d[i + q] is None else -d[i + q]), -i, n) for i in range(q)]
    for j, e in enumerate(_cfft(z, -1)):
        m = 4 * j + 1
        if m <= hf: out[m] = e
        else: out[n - m] = _conj(e)
    return out
def irfft_sym(U, n, nout):
    if n == 1: return [U[0][0]]
    if n == 2: return [_add(U[0][0], U[1][0]), _sub(U[0][0], U[1][0])][:nout]
    hf, q = n // 2, n // 4
    e = irfft_sym(U[0::2], hf, hf)
    V = []
    for j in range(q):
        m = 4 * j + 1
        V.append(U[m] if m <= hf else _conj(U[n - m]))
    w = _cfft(V, +1)
    o = [None] * hf
    for i in range(q):
        t = _ctw(w[i], i, n)
        o[i] = t[0]; o[i + q] = None if t[1] is None else -t[1]
    y = [_add(e[i], o[i]) for i in range(hf)]
    if nout > hf: y += [_sub(e[i], o[i]) for i in range(hf)]
    return y[:nout]


def _bf16_bits(a):
    u = np.ascontiguousarray(a, np.float32).view(np.uint32)
    return (u + 0x7FFF + ((u >> 16) & 1)) >> 16


def _pack_rows(a):
    b = _bf16_bits(a)
    r = b.shape[0] // 2
    return (b[:r] | (b[r:] << 16)).astype(np.uint32)


@functools.lru_cache(maxsize=None)
def _dft_consts(N1, N2, RI):
    Lf, hN = N1 * N2, N2 // 2
    k2 = np.arange(N2)[:, None]
    n2 = np.arange(N2)[None, :]
    ph = -2 * np.pi * (k2 * n2 % N2) / N2
    Fr, Fi = np.cos(ph), np.sin(ph)
    Gr, Gi = Fr.T * (2.0 / Lf), -Fi.T * (2.0 / Lf)

    def inter(a, b):
        m = np.zeros((N2, 2 * N2))
        m[:, 0::2] = a; m[:, 1::2] = b
        return m
    base = np.stack([inter(Fr, -Fi), inter(Fi, Fr), inter(Gr, -Gi), inter(Gi, Gr)]).astype(np.float32)
    th = 2 * np.pi * np.arange(N1 // 2)[:, None] * np.arange(N2)[None, :] / Lf
    twf = np.stack([np.repeat(np.cos(th), 2, axis=1), np.repeat(np.sin(th), 2, axis=1)]).astype(np.float32)
    twg = np.zeros((N2, 128), np.float32)
    twg[:, :N1 // 2] = np.cos(th).T; twg[:, 64:64 + N1 // 2] = np.sin(th).T
    f = np.zeros((2 * N2, 2 * N2))
    g = np.zeros((2 * N2, 2 * N2))
    kk = np.arange(hN)[:, None]
    p0 = -2 * np.pi * (kk * n2 % N2) / N2
    p1 = -2 * np.pi * ((kk * n2 % N2) / N2 + n2 * (N1 // 2) / Lf)
    F0r, F0i, F1r, F1i = np.cos(p0), np.sin(p0), np.cos(p1), np.sin(p1)
    nyq = np.cos(np.pi * n2[0])
    f[:hN, 0::2] = F0r; f[hN:N2, 1::2] = F1r
    f[N2:N2 + hN, 0::2] = F0i; f[N2 + hN:, 1::2] = F1i
    f[N2, 0::2] = nyq
    c = 2.0 / Lf
    g[:N2, 0:N2:2] = F0r.T * c; g[:N2, 1:N2:2] = F0i.T * c
    g[:N2, 0] = 1.0 / Lf; g[:N2, 1] = nyq / Lf
    g[N2:, N2::2] = F1r.T * c; g[N2:, N2 + 1::2] = F1i.T * c
    perm = np.arange(2 * N2).reshape(2, N2 // RI, RI).transpose(1, 0, 2).reshape(-1)
    sp = np.stack([_pack_rows(f[perm]), _pack_rows(g)])
    return base, twf, twg, sp


CFG = dict(G=2, skew_s=1, skew_pv=5, skew_wo=4, WD=256, RI=8, MS=128, MS2=128, hT="mxu", order="21AIRK", unroll=1, mi=(99, 99), flags=(),
           slots=((0, (("unroll", 2),)), (1, (("unroll", 2),)),
                  (2, (("MS", 256), ("MS2", 256))),
                  (5, (("unroll", 2), ("order", "12IAKR")))))


def _kernel(S, D, H, Dh, M, SEG, cfg,
            shift_ref, ssmD_ref, mem0_ref, gatew_ref,
            q_hbm, k_hbm, v_hbm, ssmk_hbm, wq_hbm, wk_hbm, wv_hbm, wo_hbm, cb_hbm, ctf_hbm, ctg_hbm, csp_hbm,
            out_hbm,
            x_ref, k_ref, v_ref, ssm_ref, tab_ref, cb_ref, ctf_ref, ctg_ref, shT, kv_s, hT_s, A_s, Y_s, U_s, y_ref,
            wraw, wqkv, wo, h_ref, o_ref, acc_ref, out_ref, sems, osem):
    L = M + SEG
    n_seg = S // SEG
    HP = H // 2
    WD, RI = cfg["WD"], cfg["RI"]
    N2 = 128
    NB = S // N2
    NL = WD // 128
    NBLK = D // WD

    def cp_blk(b):
        ls = pl.ds(b * WD, WD)
        return [pltpu.make_async_copy(k_hbm.at[:, ls], k_ref.at[:, ls], sems.at[3 * b]),
                pltpu.make_async_copy(v_hbm.at[:, ls], v_ref.at[:, ls], sems.at[3 * b + 1]),
                pltpu.make_async_copy(ssmk_hbm.at[ls, :], ssm_ref.at[ls, :], sems.at[3 * b + 2])]

    def wraw_copy(src, slot, sem):
        return pltpu.make_async_copy(src.bitcast(U32), wraw.at[slot], sems.at[sem])

    s0 = 3 * NBLK
    cp_c = [pltpu.make_async_copy(cb_hbm, cb_ref, sems.at[s0]),
            pltpu.make_async_copy(ctf_hbm, ctf_ref, sems.at[s0 + 1]),
            pltpu.make_async_copy(ctg_hbm, ctg_ref, sems.at[s0 + 8]),
            pltpu.make_async_copy(csp_hbm.at[0], tab_ref.at[0], sems.at[s0 + 9]),
            pltpu.make_async_copy(csp_hbm.at[1], tab_ref.at[NB], sems.at[s0 + 10])]
    cp_w = [wraw_copy(w, i, s0 + 2 + i) for i, w in enumerate((wq_hbm, wk_hbm, wv_hbm))]
    cp_wo = pltpu.make_async_copy(wo_hbm.bitcast(U32), wo, sems.at[s0 + 5])
    X0 = 4 * SEG
    cp_x0 = pltpu.make_async_copy(q_hbm.at[0:X0], x_ref.at[0:X0], sems.at[s0 + 6])
    cp_x1 = pltpu.make_async_copy(q_hbm.at[X0:], x_ref.at[X0:], sems.at[s0 + 7])
    blk_cps = [cp_blk(b) for b in range(NBLK)]
    for c in cp_c:
        c.start()
    for b in range(NBLK):
        for c in blk_cps[b]:
            c.start()
    late = cp_w + [cp_x0, cp_wo, cp_x1]
    w_start = cfg.get("w_start", (0, 0, 0, 0, 0, 0))
    for c, sl in zip(late, w_start):
        if sl == 0:
            c.start()

    shT[...] = jnp.concatenate(
        [shift_ref[...].astype(F32), jnp.zeros((D, 128 - shift_ref.shape[1]), F32)], axis=1).T[:8]
    ks_taps = shift_ref.shape[1]
    eye = (jax.lax.broadcasted_iota(jnp.int32, (N2, N2), 0)
           == jax.lax.broadcasted_iota(jnp.int32, (N2, N2), 1)).astype(BF16)

    for c in cp_c:
        c.wait()
    hq = N2 // 2
    for k1 in range(1, NB):
        cf, sf = ctf_ref[0, k1:k1 + 1, :], ctf_ref[1, k1:k1 + 1, :]
        for q in range(N2 // 8):
            g8 = (q // 2) * 8

            def rot(r):
                fre, fim = cb_ref[0, r:r + 8, :], cb_ref[1, r:r + 8, :]
                return fre * cf + fim * sf if q % 2 == 0 else fim * cf - fre * sf
            tab_ref[k1, q * 8:q * 8 + 8, :] = pltpu.pack_elementwise([rot(g8), rot(hq + g8)], packed_dtype=BF16)
            rows = slice(q * 8, q * 8 + 8)
            cg = jnp.broadcast_to(ctg_ref[rows, k1:k1 + 1], (8, 2 * N2))
            sg = jnp.broadcast_to(ctg_ref[rows, 64 + k1:64 + k1 + 1], (8, 2 * N2))
            gre, gim = cb_ref[2, rows, :], cb_ref[3, rows, :]
            tab_ref[NB + k1, rows, :] = pltpu.pack_elementwise(
                [gre * cg - gim * sg, gim * cg + gre * sg], packed_dtype=BF16)

    def st_kv(b, i):
        r0 = pl.multiple_of(i * N2, N2)
        rp = pl.multiple_of(jnp.maximum(r0 - 16, 0), 16)
        for j in range(NL):
            lg = pl.ds(b * WD + j * 128, 128)
            ll = pl.ds(j * 128, 128)
            cur = k_ref[pl.ds(r0, N2), lg].astype(F32)
            prev = jnp.where(i > 0, k_ref[pl.ds(rp, 16), lg].astype(F32), 0.0)
            ext = jnp.concatenate([prev[8:16], cur], axis=0)
            w = shT[:, lg]
            ks = cur * w[0:1]
            for t in range(1, ks_taps):
                ks = ks + ext[8 - t:8 - t + N2] * w[t:t + 1]
            kv = ks * v_ref[pl.ds(r0, N2), lg].astype(F32)
            kv_s[b % 2, pl.ds(r0, N2), ll] = kv
            y_ref[pl.ds(r0, N2), lg] = kv * ssmD_ref[:, lg].astype(F32)
            if cfg["hT"] == "xlu":
                hT_s[b % 2, pl.ds(r0, N2), ll] = ssm_ref[lg, pl.ds(r0, N2)].astype(F32).T
            else:
                hT_s[b % 2, pl.ds(r0, N2), ll] = jax.lax.dot_general(
                    eye, ssm_ref[lg, pl.ds(r0, N2)], (((1,), (1,)), ((), ())), preferred_element_type=F32)
            yield

    def st_a(b, i):
        r0 = pl.multiple_of(i * 8, 8)
        for src, off in ((kv_s, 0), (hT_s, 128)):
            for j in range(NL):
                xs = [src[b % 2, pl.ds(n1 * N2 + r0, 8), pl.ds(j * 128, 128)] for n1 in range(NB)]
                X = rfft_sym(xs + [None] * NB)
                for k1 in range(NB):
                    pair = [X[0][0], X[NB][0]] if k1 == 0 else [X[k1][0], X[k1][1]]
                    A_s[b % 2, k1, pl.ds(r0, 8), pl.ds(off + j * 256, 128)] = (
                        pltpu.pack_elementwise(pair, packed_dtype=BF16))
                yield

    def table(idx):
        w = tab_ref[idx]
        return jnp.concatenate([pltpu.bitcast(w << 16, F32),
                                pltpu.bitcast(w & np.uint32(0xFFFF0000), F32)], axis=0)

    def mm(a, b):
        return jax.lax.dot_general(a, b, (((1,), (0,)), ((), ())), preferred_element_type=F32)

    def st_g1(b, i, par):
        Fm = table(i)
        MS = cfg["MS"]
        for j in range(NL):
            Am = pltpu.bitcast(A_s[b % 2, i, :, pl.ds(j * 256, 256)], BF16)
            for m0 in range(0, 2 * N2, MS):
                X = mm(Fm[m0:m0 + MS], Am)
                for r in range(MS // (2 * RI)):
                    re = X[2 * r * RI:(2 * r + 1) * RI]
                    im = X[(2 * r + 1) * RI:(2 * r + 2) * RI]
                    a, c = re[:, :128], re[:, 128:]
                    b_, d = im[:, :128], im[:, 128:]
                    bd = b_ * d
                    yre, yim = a * c - bd, a * d + b_ * c
                    row = m0 // 2 + r * RI
                    if row == 0:
                        rid = jax.lax.broadcasted_iota(jnp.int32, (RI, 128), 0) + i
                        yre = jnp.where(rid == 0, a * c, yre)
                        yim = jnp.where(rid == 0, bd, yim)
                    Y_s[par, pl.ds(row, RI), pl.ds(j * 128, 128)] = (
                        pltpu.pack_elementwise([yre, yim], packed_dtype=BF16))
                yield

    def st_g2(b, i, par):
        Gm = table(NB + i)
        MS = cfg["MS2"]
        Ym = pltpu.bitcast(Y_s[par], BF16)
        for m0 in range(0, 2 * N2, MS):
            U_s[b % 2, i, pl.ds(m0, MS), :] = mm(Gm[m0:m0 + MS], Ym)
            yield

    def st_i(b, i):
        r0 = pl.multiple_of(i * 8, 8)
        for j in range(NL):
            lg = pl.ds(b * WD + j * 128, 128)
            ld = lambda k1, part: U_s[b % 2, k1, pl.ds(part * N2 + r0, 8), pl.ds(j * 128, 128)]
            U = [(ld(0, 0), None)] + [(ld(k1, 0), ld(k1, 1)) for k1 in range(1, NB)] + [(ld(0, 1), None)]
            ys = irfft_sym(U, 2 * NB, NB)
            for n1 in range(NB):
                rr = pl.ds(n1 * N2 + r0, 8)
                y_ref[rr, lg] = y_ref[rr, lg] + ys[n1]
            yield

    def st_relayout(slot, i, n_per):
        for u in range(n_per):
            ii = i * n_per + u
            r0 = pl.multiple_of(ii * 8, 8)
            raw = wraw.at[slot].reshape(D * HP, Dh)
            for hp in range(HP):
                a = raw[pl.ds(ii * 16 * HP + hp, 8, stride=2 * HP), :]
                b = raw[pl.ds(ii * 16 * HP + HP + hp, 8, stride=2 * HP), :]
                c0 = (2 * hp) * 3 * Dh + slot * Dh
                wqkv[pl.ds(r0, 8), pl.ds(c0, Dh)] = (a & 0xFFFF) | (b << 16)
                wqkv[pl.ds(r0, 8), pl.ds(c0 + 3 * Dh, Dh)] = (a >> 16) | (b & np.uint32(0xFFFF0000))
            yield

    rel_slot = cfg.get("rel_slot", (NBLK - 1, NBLK, NBLK + 1))
    n_slots = max(NBLK + 3, max(rel_slot) + 1)
    cfg = dict(cfg)
    cfg0 = dict(cfg)
    for slot in range(n_slots):
        cfg.update(cfg0)
        cfg.update(dict(dict(cfg0["slots"]).get(slot, ())))
        bk, ba, bg, bi = slot, slot - 1, slot - 2, slot - 3
        ok = lambda b: 0 <= b < NBLK
        scope = contextlib.ExitStack()
        if cfg0.get("prof"):
            scope.enter_context(jax.named_scope(f"wait{slot}"))
        if ok(bk):
            for c in blk_cps[bk]:
                c.wait()
        for c, sl in zip(late, w_start):
            if sl == slot and sl > 0:
                c.start()
        rel = [m for m in range(3) if rel_slot[m] == slot]
        for m in rel:
            cp_w[m].wait()
        scope.close()
        if cfg0.get("prof"):
            scope.enter_context(jax.named_scope(f"slot{slot}"))

        def body1(i, par, first=False, bk=bk, ba=ba, bg=bg, bi=bi, rel=rel):
            def chain(gens):
                for g_ in gens:
                    yield from g_
            mxu, vpu = [], []
            for st in cfg["order"]:
                if st == "1" and ok(bg):
                    mxu.append(st_g1(bg, i, par))
                elif st == "2" and ok(bg) and not first:
                    mxu.append(st_g2(bg, i - 1, 1 - par))
                elif st == "I" and ok(bi):
                    vpu.append(st_i(bi, i))
                elif st == "A" and ok(ba):
                    vpu.append(st_a(ba, i))
                elif st == "K" and ok(bk):
                    vpu.append(st_kv(bk, i))
                elif st == "R":
                    vpu.extend(st_relayout(m, i, D // 16 // NB) for m in rel)
            mg, vg = chain(mxu), chain(vpu)
            done = object()
            alive = [True, True]
            while any(alive):
                for n_, (g_, rep) in enumerate(((mg, cfg["mi"][0]), (vg, cfg["mi"][1]))):
                    for _ in range(rep):
                        if alive[n_] and next(g_, done) is done:
                            alive[n_] = False

        UN = cfg["unroll"]

        def body(i0, carry):
            for u in range(UN):
                body1(i0 * UN + u, u % 2 if UN > 1 else (i0 % 2))
            return carry

        if ok(bg):
            for u in range(UN):
                body1(u, u % 2, first=(u == 0))
            jax.lax.fori_loop(1, NB // UN, body, 0)
            for _ in st_g2(bg, NB - 1, (NB - 1) % 2):
                pass
        else:
            jax.lax.fori_loop(0, NB // UN, body, 0)
        scope.close()

    cfg.update(cfg0)
    cp_x0.wait()
    cp_wo.wait()

    scale = Dh ** (-0.5)
    G = cfg["G"]
    gate_w = gatew_ref[...].astype(F32)

    def step(s, mem):
        r0 = pl.multiple_of(s * SEG, SEG)
        xs = x_ref[pl.ds(r0, SEG), :].astype(F32)
        h_ref[0:M, :] = mem
        h_ref[M:L, :] = xs
        row = jax.lax.broadcasted_iota(jnp.int32, (L, L), 0)
        col = jax.lax.broadcasted_iota(jnp.int32, (L, L), 1)
        mask = (row < M) | (row >= col)

        qkv = {}
        probs = {}

        def proj(h):
            w = pltpu.bitcast(wqkv[:, pl.ds(h * 3 * Dh, 3 * Dh)], BF16)
            r = jax.lax.dot_general(h_ref[...], w, (((1,), (0,)), ((), ())),
                                    preferred_element_type=F32)
            qkv[h] = (r[:, :Dh], r[:, Dh:2 * Dh].astype(BF16), r[:, 2 * Dh:].astype(BF16))

        def scores(h):
            q, k, _ = qkv[h]
            sc = jax.lax.dot_general(q, k, (((1,), (1,)), ((), ())),
                                     preferred_element_type=F32) * scale
            sc = jnp.where(mask, sc, -1e9)
            m = jnp.max(sc, axis=-1, keepdims=True)
            e = jnp.exp(sc - m)
            probs[h] = e / jnp.sum(e, axis=-1, keepdims=True)

        def pv(h):
            o = jnp.dot(probs.pop(h), qkv.pop(h)[2], preferred_element_type=F32)
            o_ref[:, pl.ds(h * Dh, Dh)] = o

        def wo_group(g):
            w = pltpu.bitcast(wo[pl.ds(g * G * Dh // 2, G * Dh // 2), :], BF16)
            r = jax.lax.dot_general(o_ref[:, pl.ds(g * G * Dh, G * Dh)], w,
                                    (((1,), (0,)), ((), ())), preferred_element_type=F32)
            if g == 0:
                acc_ref[...] = r
            elif g < H // G - 1:
                acc_ref[...] += r
            else:
                return acc_ref[...] + r

        s1, s2, s3 = cfg["skew_s"], cfg["skew_pv"], cfg["skew_wo"]
        res = None
        for t in range(H + s1 + s2 + s3):
            if t < H:
                proj(t)
            if 0 <= t - s1 < H:
                scores(t - s1)
            hh = t - s1 - s2
            if 0 <= hh < H:
                pv(hh)
            hw = t - s1 - s2 - s3
            if 0 <= hw < H and (hw + 1) % G == 0:
                res = wo_group(hw // G)
        mem_next = res[0:M, :].astype(BF16).astype(F32)
        b = res[M:L, :]
        g = jax.nn.sigmoid(jnp.sum(xs * gate_w, axis=-1, keepdims=True))
        a = xs * y_ref[pl.ds(r0, SEG), :]
        out_ref[pl.ds(r0, SEG), :] = (g * a + (1.0 - g) * b).astype(out_ref.dtype)
        pltpu.make_async_copy(out_ref.at[pl.ds(r0, SEG)], out_hbm.at[pl.ds(r0, SEG)], osem).start()
        return mem_next

    nst = cfg.get("nsteps", n_seg)
    n1 = X0 // SEG
    mem = jax.lax.fori_loop(0, n1, step, mem0_ref[...].astype(F32))
    cp_x1.wait()
    jax.lax.fori_loop(n1, nst, step, mem)
    pltpu.make_async_copy(out_ref.at[0:nst * SEG], out_hbm.at[0:nst * SEG], osem).wait()


@functools.partial(jax.jit, static_argnames=("B_seg_len", "cfg"))
def pallas_gated_mix__ssm_conv_h3__memory_aug_recurrent_mem_tr__prompt_kernel(
    A_q, A_k, A_v, A_shift_k, A_ssm_k, A_ssm_D, B_x, B_mem0, B_Wq, B_Wk, B_Wv, B_Wo,
    B_seg_len, gate_w, cfg=None,
):
    del B_x
    cfg = dict(CFG, **dict(cfg or ()))
    _, S, D = A_q.shape
    _, H, Dh = B_Wq.shape
    M = B_mem0.shape[1]
    SEG = int(B_seg_len)
    L = M + SEG
    WD = cfg["WD"]
    NB = S // 128
    assert cfg["RI"] == 8
    consts = _dft_consts(2 * NB, 128, cfg["RI"])
    kern = functools.partial(_kernel, S, D, H, Dh, M, SEG, cfg)
    vm = pl.BlockSpec(memory_space=pltpu.VMEM)
    hbm = pl.BlockSpec(memory_space=pl.ANY)
    out = pl.pallas_call(
        kern,
        out_shape=jax.ShapeDtypeStruct((S, D), BF16),
        in_specs=[vm, vm, vm, vm] + [hbm] * 12,
        out_specs=hbm,
        scratch_shapes=[
            pltpu.VMEM((S, D), BF16),
            pltpu.VMEM((S, D), BF16),
            pltpu.VMEM((S, D), BF16),
            pltpu.VMEM((D, S), BF16),
            pltpu.VMEM((2 * NB, 128, 256), U32),
            pltpu.VMEM(consts[0].shape, F32),
            pltpu.VMEM(consts[1].shape, F32),
            pltpu.VMEM(consts[2].shape, F32),
            pltpu.VMEM((8, D), F32),
            pltpu.VMEM((2, S, WD), F32),
            pltpu.VMEM((2, S, WD), F32),
            pltpu.VMEM((2, NB, 128, 2 * WD), U32),
            pltpu.VMEM((2, 128, WD), U32),
            pltpu.VMEM((2, NB, 256, WD), F32),
            pltpu.VMEM((S, D), F32),
            pltpu.VMEM((3, D, H // 2, Dh), U32),
            pltpu.VMEM((D // 2, 3 * H * Dh), U32),
            pltpu.VMEM((H * Dh // 2, D), U32),
            pltpu.VMEM((L, D), F32),
            pltpu.VMEM((L, H * Dh), F32),
            pltpu.VMEM((L, D), F32),
            pltpu.VMEM((S, D), BF16),
            pltpu.SemaphoreType.DMA((3 * (D // WD) + 11,)),
            pltpu.SemaphoreType.DMA,
        ],
        compiler_params=pltpu.CompilerParams(
            vmem_limit_bytes=120 * 1024 * 1024, flags=dict(cfg["flags"]) or None),
    )(
        A_shift_k, A_ssm_D.reshape(1, D), B_mem0.reshape(M, D), gate_w.reshape(1, D),
        A_q.reshape(S, D), A_k.reshape(S, D), A_v.reshape(S, D), A_ssm_k,
        B_Wq, B_Wk, B_Wv, B_Wo.reshape(H * Dh, D), *consts,
    )
    return out.reshape(1, S, D)
```

```python
import contextlib
import functools
import math

import numpy as np
import jax
import jax.numpy as jnp
import jax.experimental.pallas as pl
import jax.experimental.pallas.tpu as pltpu

F32 = jnp.float32
BF16 = jnp.bfloat16
U32 = jnp.uint32

def _neg(a):
    return None if a is None else (-a[0], a[1])
def _add(a, b):
    if a is None or b is None:
        return b if a is None else a
    if a[0] == b[0]:
        return (a[0], a[1] + b[1])
    return (1, a[1] - b[1]) if a[0] > 0 else (1, b[1] - a[1])
def _sub(a, b):
    return _add(a, _neg(b))
def _val(a):
    return a[1] if a[0] > 0 else -a[1]
def _cadd(a, b): return (_add(a[0], b[0]), _add(a[1], b[1]))
def _csub(a, b): return (_sub(a[0], b[0]), _sub(a[1], b[1]))
def _mulc(a, c):
    if a is None or abs(c) < 1e-12: return None
    if abs(c - 1) < 1e-12: return a
    if abs(c + 1) < 1e-12: return _neg(a)
    return (1, a[1] * np.float32(c * a[0]))
def _ctw(z, num, den):
    num %= den
    re, im = z
    if (4 * num) % den == 0:
        qd = (4 * num) // den
        return [(re, im), (_neg(im), re), (_neg(re), _neg(im)), (im, _neg(re))][qd]
    c, s = math.cos(2 * math.pi * num / den), math.sin(2 * math.pi * num / den)
    if (8 * num) % den == 0 and re is not None and im is not None:
        if c * s > 0:
            return (_mulc(_sub(re, im), c), _mulc(_add(im, re), c))
        return (_mulc(_add(re, im), c), _mulc(_sub(im, re), c))
    return (_sub(_mulc(re, c), _mulc(im, s)), _add(_mulc(re, s), _mulc(im, c)))
def _cfft(zs, sign):
    n = len(zs)
    if n == 1: return list(zs)
    ev, od = _cfft(zs[0::2], sign), _cfft(zs[1::2], sign)
    out = [None] * n
    for j in range(n // 2):
        t = _ctw(od[j], sign * j, n)
        out[j] = _cadd(ev[j], t); out[j + n // 2] = _csub(ev[j], t)
    return out
def _conj(z): return (z[0], _neg(z[1]))
def rfft_sym(xs):
    n = len(xs)
    if n == 1: return [(xs[0], None)]
    if n == 2: return [(_add(xs[0], xs[1]), None), (_sub(xs[0], xs[1]), None)]
    hf, q = n // 2, n // 4
    s = [_add(xs[i], xs[i + hf]) for i in range(hf)]
    d = [_sub(xs[i], xs[i + hf]) for i in range(hf)]
    out = [None] * (hf + 1)
    for j, e in enumerate(rfft_sym(s)): out[2 * j] = e
    z = [_ctw((d[i], _neg(d[i + q])), -i, n) for i in range(q)]
    for j, e in enumerate(_cfft(z, -1)):
        m = 4 * j + 1
        if m <= hf: out[m] = e
        else: out[n - m] = _conj(e)
    return out
def irfft_sym(U, n, nout):
    if n == 1: return [U[0][0]]
    if n == 2: return [_add(U[0][0], U[1][0]), _sub(U[0][0], U[1][0])][:nout]
    hf, q = n // 2, n // 4
    e = irfft_sym(U[0::2], hf, hf)
    V = []
    for j in range(q):
        m = 4 * j + 1
        V.append(U[m] if m <= hf else _conj(U[n - m]))
    w = _cfft(V, +1)
    o = [None] * hf
    for i in range(q):
        t = _ctw(w[i], i, n)
        o[i] = t[0]; o[i + q] = _neg(t[1])
    y = [_add(e[i], o[i]) for i in range(hf)]
    if nout > hf: y += [_sub(e[i], o[i]) for i in range(hf)]
    return y[:nout]


def _bf16_bits(a):
    u = np.ascontiguousarray(a, np.float32).view(np.uint32)
    return (u + 0x7FFF + ((u >> 16) & 1)) >> 16


def _pack_rows(a):
    b = _bf16_bits(a)
    r = b.shape[0] // 2
    return (b[:r] | (b[r:] << 16)).astype(np.uint32)


@functools.lru_cache(maxsize=None)
def _dft_consts(N1, N2, RI):
    Lf, hN = N1 * N2, N2 // 2
    k2 = np.arange(N2)[:, None]
    n2 = np.arange(N2)[None, :]
    ph = -2 * np.pi * (k2 * n2 % N2) / N2
    Fr, Fi = np.cos(ph), np.sin(ph)
    Gr, Gi = Fr.T * (2.0 / Lf), -Fi.T * (2.0 / Lf)

    def inter(a, b):
        m = np.zeros((N2, 2 * N2))
        m[:, 0::2] = a; m[:, 1::2] = b
        return m
    base = np.stack([inter(Fr, -Fi), inter(Fi, Fr), inter(Gr, -Gi), inter(Gi, Gr)]).astype(np.float32)
    th = 2 * np.pi * np.arange(N1 // 2)[:, None] * np.arange(N2)[None, :] / Lf
    twf = np.stack([np.repeat(np.cos(th), 2, axis=1), np.repeat(np.sin(th), 2, axis=1)]).astype(np.float32)
    twg = np.zeros((N2, 128), np.float32)
    twg[:, :N1 // 2] = np.cos(th).T; twg[:, 64:64 + N1 // 2] = np.sin(th).T
    f = np.zeros((2 * N2, 2 * N2))
    g = np.zeros((2 * N2, 2 * N2))
    kk = np.arange(hN)[:, None]
    p0 = -2 * np.pi * (kk * n2 % N2) / N2
    p1 = -2 * np.pi * ((kk * n2 % N2) / N2 + n2 * (N1 // 2) / Lf)
    F0r, F0i, F1r, F1i = np.cos(p0), np.sin(p0), np.cos(p1), np.sin(p1)
    nyq = np.cos(np.pi * n2[0])
    f[:hN, 0::2] = F0r; f[hN:N2, 1::2] = F1r
    f[N2:N2 + hN, 0::2] = F0i; f[N2 + hN:, 1::2] = F1i
    f[N2, 0::2] = nyq
    c = 2.0 / Lf
    g[:N2, 0:N2:2] = F0r.T * c; g[:N2, 1:N2:2] = F0i.T * c
    g[:N2, 0] = 1.0 / Lf; g[:N2, 1] = nyq / Lf
    g[N2:, N2::2] = F1r.T * c; g[N2:, N2 + 1::2] = F1i.T * c
    perm = np.arange(2 * N2).reshape(2, N2 // RI, RI).transpose(1, 0, 2).reshape(-1)
    sp = np.stack([_pack_rows(f[perm]), _pack_rows(g)])
    return base, twf, twg, sp


CFG = dict(G=1, skew_s=1, skew_pv=5, skew_wo=4, WD=256, RI=8, MS=128, MS2=128, hT="mxu", order="21AIRK", unroll=1, mi=(99, 99), flags=(), su=2,
           slots=((0, (("unroll", 2),)), (1, (("unroll", 2),)),
                  (2, (("MS", 256), ("MS2", 256))),
                  (5, (("unroll", 2), ("order", "12IAKR")))))


def _kernel(S, D, H, Dh, M, SEG, cfg,
            shift_ref, ssmD_ref, mem0_ref, gatew_ref,
            q_hbm, k_hbm, v_hbm, ssmk_hbm, wq_hbm, wk_hbm, wv_hbm, wo_hbm, cb_hbm, ctf_hbm, ctg_hbm, csp_hbm,
            out_hbm,
            x_ref, k_ref, v_ref, ssm_ref, tab_ref, cb_ref, ctf_ref, ctg_ref, shT, kv_s, hT_s, A_s, Y_s, U_s, y_ref,
            wraw, wqkv, wo, h_ref, o_ref, acc_ref, out_ref, sems, osem):
    L = M + SEG
    n_seg = S // SEG
    HP = H // 2
    WD, RI = cfg["WD"], cfg["RI"]
    N2 = 128
    NB = S // N2
    NL = WD // 128
    NBLK = D // WD

    def cp_blk(b):
        ls = pl.ds(b * WD, WD)
        return [pltpu.make_async_copy(k_hbm.at[:, ls], k_ref.at[:, ls], sems.at[3 * b]),
                pltpu.make_async_copy(v_hbm.at[:, ls], v_ref.at[:, ls], sems.at[3 * b + 1]),
                pltpu.make_async_copy(ssmk_hbm.at[ls, :], ssm_ref.at[ls, :], sems.at[3 * b + 2])]

    def wraw_copy(src, slot, sem):
        return pltpu.make_async_copy(src.bitcast(U32), wraw.at[slot], sems.at[sem])

    s0 = 3 * NBLK
    cp_c = [pltpu.make_async_copy(cb_hbm, cb_ref, sems.at[s0]),
            pltpu.make_async_copy(ctf_hbm, ctf_ref, sems.at[s0 + 1]),
            pltpu.make_async_copy(ctg_hbm, ctg_ref, sems.at[s0 + 8]),
            pltpu.make_async_copy(csp_hbm.at[0], tab_ref.at[0], sems.at[s0 + 9]),
            pltpu.make_async_copy(csp_hbm.at[1], tab_ref.at[NB], sems.at[s0 + 10])]
    cp_w = [wraw_copy(w, i, s0 + 2 + i) for i, w in enumerate((wq_hbm, wk_hbm, wv_hbm))]
    cp_wo = pltpu.make_async_copy(wo_hbm.bitcast(U32), wo, sems.at[s0 + 5])
    cp_x = pltpu.make_async_copy(q_hbm, x_ref, sems.at[s0 + 6])
    blk_cps = [cp_blk(b) for b in range(NBLK)]
    for c in cp_c:
        c.start()
    for b in range(NBLK):
        for c in blk_cps[b]:
            c.start()
    late = cp_w + [cp_wo, cp_x]
    w_start = cfg.get("w_start", (0, 0, 0, 0, 0))
    for c, sl in zip(late, w_start):
        if sl == 0:
            c.start()

    ks_taps = shift_ref.shape[0]
    shT[0:ks_taps, :] = shift_ref[...].astype(F32)
    shT[ks_taps:ks_taps + 1, :] = ssmD_ref[...].astype(F32).reshape(1, D)
    eye = (jax.lax.broadcasted_iota(jnp.int32, (N2, N2), 0)
           == jax.lax.broadcasted_iota(jnp.int32, (N2, N2), 1)).astype(BF16)

    for c in cp_c:
        c.wait()
    hq = N2 // 2
    for k1 in range(1, NB):
        cf, sf = ctf_ref[0, k1:k1 + 1, :], ctf_ref[1, k1:k1 + 1, :]
        for q in range(N2 // 8):
            g8 = (q // 2) * 8

            def rot(r):
                fre, fim = cb_ref[0, r:r + 8, :], cb_ref[1, r:r + 8, :]
                return fre * cf + fim * sf if q % 2 == 0 else fim * cf - fre * sf
            tab_ref[k1, q * 8:q * 8 + 8, :] = pltpu.pack_elementwise([rot(g8), rot(hq + g8)], packed_dtype=BF16)
            rows = slice(q * 8, q * 8 + 8)
            cg = jnp.broadcast_to(ctg_ref[rows, k1:k1 + 1], (8, 2 * N2))
            sg = jnp.broadcast_to(ctg_ref[rows, 64 + k1:64 + k1 + 1], (8, 2 * N2))
            gre, gim = cb_ref[2, rows, :], cb_ref[3, rows, :]
            tab_ref[NB + k1, rows, :] = pltpu.pack_elementwise(
                [gre * cg - gim * sg, gim * cg + gre * sg], packed_dtype=BF16)

    def st_kv(b, i):
        r0 = pl.multiple_of(i * N2, N2)
        rp = pl.multiple_of(jnp.maximum(r0 - 16, 0), 16)
        for j in range(NL):
            lg = pl.ds(b * WD + j * 128, 128)
            ll = pl.ds(j * 128, 128)
            cur = k_ref[pl.ds(r0, N2), lg].astype(F32)
            prev = jnp.where(i > 0, k_ref[pl.ds(rp, 16), lg].astype(F32), 0.0)
            ext = jnp.concatenate([prev[8:16], cur], axis=0)
            w = shT[0:ks_taps + 1, lg]
            ks = cur * w[0:1]
            for t in range(1, ks_taps):
                ks = ks + ext[8 - t:8 - t + N2] * w[t:t + 1]
            kv = ks * v_ref[pl.ds(r0, N2), lg].astype(F32)
            kv_s[b % 2, pl.ds(r0, N2), ll] = kv
            y_ref[pl.ds(r0, N2), lg] = kv * w[ks_taps:ks_taps + 1]
            if cfg["hT"] == "xlu":
                hT_s[b % 2, pl.ds(r0, N2), ll] = ssm_ref[lg, pl.ds(r0, N2)].astype(F32).T
            else:
                hT_s[b % 2, pl.ds(r0, N2), ll] = jax.lax.dot_general(
                    eye, ssm_ref[lg, pl.ds(r0, N2)], (((1,), (1,)), ((), ())), preferred_element_type=F32)
            yield

    def st_a(b, i):
        r0 = pl.multiple_of(i * 8, 8)
        for src, off in ((kv_s, 0), (hT_s, 128)):
            for j in range(NL):
                xs = [src[b % 2, pl.ds(n1 * N2 + r0, 8), pl.ds(j * 128, 128)] for n1 in range(NB)]
                X = rfft_sym([(1, x) for x in xs] + [None] * NB)
                for k1 in range(NB):
                    pair = [X[0][0], X[NB][0]] if k1 == 0 else [X[k1][0], X[k1][1]]
                    pair = [_val(t) for t in pair]
                    A_s[b % 2, k1, pl.ds(r0, 8), pl.ds(off + j * 256, 128)] = (
                        pltpu.pack_elementwise(pair, packed_dtype=BF16))
                yield

    def table(idx):
        w = tab_ref[idx]
        return jnp.concatenate([pltpu.bitcast(w << 16, F32),
                                pltpu.bitcast(w & np.uint32(0xFFFF0000), F32)], axis=0)

    def mm(a, b):
        return jax.lax.dot_general(a, b, (((1,), (0,)), ((), ())), preferred_element_type=F32)

    def st_g1(b, i, par):
        Fm = table(i)
        MS = cfg["MS"]
        for j in range(NL):
            Am = pltpu.bitcast(A_s[b % 2, i, :, pl.ds(j * 256, 256)], BF16)
            for m0 in range(0, 2 * N2, MS):
                X = mm(Fm[m0:m0 + MS], Am)
                for r in range(MS // (2 * RI)):
                    re = X[2 * r * RI:(2 * r + 1) * RI]
                    im = X[(2 * r + 1) * RI:(2 * r + 2) * RI]
                    a, c = re[:, :128], re[:, 128:]
                    b_, d = im[:, :128], im[:, 128:]
                    bd = b_ * d
                    yre, yim = a * c - bd, a * d + b_ * c
                    row = m0 // 2 + r * RI
                    if row == 0:
                        rid = jax.lax.broadcasted_iota(jnp.int32, (RI, 128), 0) + i
                        yre = jnp.where(rid == 0, a * c, yre)
                        yim = jnp.where(rid == 0, bd, yim)
                    Y_s[par, pl.ds(row, RI), pl.ds(j * 128, 128)] = (
                        pltpu.pack_elementwise([yre, yim], packed_dtype=BF16))
                yield

    def st_g2(b, i, par):
        Gm = table(NB + i)
        MS = cfg["MS2"]
        Ym = pltpu.bitcast(Y_s[par], BF16)
        for m0 in range(0, 2 * N2, MS):
            U_s[b % 2, i, pl.ds(m0, MS), :] = mm(Gm[m0:m0 + MS], Ym)
            yield

    def st_i(b, i):
        r0 = pl.multiple_of(i * 8, 8)
        for j in range(NL):
            lg = pl.ds(b * WD + j * 128, 128)
            ld = lambda k1, part: (1, U_s[b % 2, k1, pl.ds(part * N2 + r0, 8), pl.ds(j * 128, 128)])
            U = [(ld(0, 0), None)] + [(ld(k1, 0), ld(k1, 1)) for k1 in range(1, NB)] + [(ld(0, 1), None)]
            ys = irfft_sym(U, 2 * NB, NB)
            for n1 in range(NB):
                rr = pl.ds(n1 * N2 + r0, 8)
                y_ref[rr, lg] = _val(_add((1, y_ref[rr, lg]), ys[n1]))
            yield

    def st_relayout(slot, i, n_per):
        for u in range(n_per):
            ii = i * n_per + u
            r0 = pl.multiple_of(ii * 8, 8)
            raw = wraw.at[slot].reshape(D * HP, Dh)
            for hp in range(HP):
                a = raw[pl.ds(ii * 16 * HP + hp, 8, stride=2 * HP), :]
                b = raw[pl.ds(ii * 16 * HP + HP + hp, 8, stride=2 * HP), :]
                c0 = (2 * hp) * 3 * Dh + slot * Dh
                wqkv[pl.ds(r0, 8), pl.ds(c0, Dh)] = (a & 0xFFFF) | (b << 16)
                wqkv[pl.ds(r0, 8), pl.ds(c0 + 3 * Dh, Dh)] = (a >> 16) | (b & np.uint32(0xFFFF0000))
            yield

    rel_slot = cfg.get("rel_slot", (NBLK - 1, NBLK, NBLK + 1))
    n_slots = max(NBLK + 3, max(rel_slot) + 1)
    cfg = dict(cfg)
    cfg0 = dict(cfg)
    for slot in range(n_slots):
        cfg.update(cfg0)
        cfg.update(dict(dict(cfg0["slots"]).get(slot, ())))
        bk, ba, bg, bi = slot, slot - 1, slot - 2, slot - 3
        ok = lambda b: 0 <= b < NBLK
        scope = contextlib.ExitStack()
        if cfg0.get("prof"):
            scope.enter_context(jax.named_scope(f"wait{slot}"))
        if ok(bk):
            for c in blk_cps[bk]:
                c.wait()
        for c, sl in zip(late, w_start):
            if sl == slot and sl > 0:
                c.start()
        rel = [m for m in range(3) if rel_slot[m] == slot]
        for m in rel:
            cp_w[m].wait()
        scope.close()
        if cfg0.get("prof"):
            scope.enter_context(jax.named_scope(f"slot{slot}"))

        def body1(i, par, first=False, bk=bk, ba=ba, bg=bg, bi=bi, rel=rel):
            def chain(gens):
                for g_ in gens:
                    yield from g_
            mxu, vpu = [], []
            for st in cfg["order"]:
                if st == "1" and ok(bg):
                    mxu.append(st_g1(bg, i, par))
                elif st == "2" and ok(bg) and not first:
                    mxu.append(st_g2(bg, i - 1, 1 - par))
                elif st == "I" and ok(bi):
                    vpu.append(st_i(bi, i))
                elif st == "A" and ok(ba):
                    vpu.append(st_a(ba, i))
                elif st == "K" and ok(bk):
                    vpu.append(st_kv(bk, i))
                elif st == "R":
                    vpu.extend(st_relayout(m, i, D // 16 // NB) for m in rel)
            mg, vg = chain(mxu), chain(vpu)
            done = object()
            alive = [True, True]
            while any(alive):
                for n_, (g_, rep) in enumerate(((mg, cfg["mi"][0]), (vg, cfg["mi"][1]))):
                    for _ in range(rep):
                        if alive[n_] and next(g_, done) is done:
                            alive[n_] = False

        UN = cfg["unroll"]

        def body(i0, carry):
            for u in range(UN):
                body1(i0 * UN + u, u % 2 if UN > 1 else (i0 % 2))
            return carry

        if ok(bg):
            for u in range(UN):
                body1(u, u % 2, first=(u == 0))
            jax.lax.fori_loop(1, NB // UN, body, 0)
            for _ in st_g2(bg, NB - 1, (NB - 1) % 2):
                pass
        else:
            jax.lax.fori_loop(0, NB // UN, body, 0)
        scope.close()

    cfg.update(cfg0)
    cp_wo.wait()
    cp_x.wait()

    scale = Dh ** (-0.5)
    G = cfg["G"]
    gate_w = gatew_ref[...].astype(F32).reshape(1, D)

    def step(s, mem):
        r0 = pl.multiple_of(s * SEG, SEG)
        xs = x_ref[pl.ds(r0, SEG), :].astype(F32)
        h_ref[0:M, :] = mem
        h_ref[M:L, :] = xs
        row = jax.lax.broadcasted_iota(jnp.int32, (L, L), 0)
        col = jax.lax.broadcasted_iota(jnp.int32, (L, L), 1)
        mask = (row < M) | (row >= col)

        qkv = {}
        probs = {}

        def proj(h):
            w = pltpu.bitcast(wqkv[:, pl.ds(h * 3 * Dh, 3 * Dh)], BF16)
            r = jax.lax.dot_general(h_ref[...], w, (((1,), (0,)), ((), ())),
                                    preferred_element_type=F32)
            qkv[h] = (r[:, :Dh], r[:, Dh:2 * Dh].astype(BF16), r[:, 2 * Dh:].astype(BF16))

        def scores(h):
            q, k, _ = qkv[h]
            sc = jax.lax.dot_general(q, k, (((1,), (1,)), ((), ())),
                                     preferred_element_type=F32) * scale
            sc = jnp.where(mask, sc, -1e9)
            m = jnp.max(sc, axis=-1, keepdims=True)
            e = jnp.exp(sc - m)
            probs[h] = e / jnp.sum(e, axis=-1, keepdims=True)

        def pv(h):
            o = jnp.dot(probs.pop(h), qkv.pop(h)[2], preferred_element_type=F32)
            o_ref[:, pl.ds(h * Dh, Dh)] = o

        def wo_group(g):
            w = pltpu.bitcast(wo[pl.ds(g * G * Dh // 2, G * Dh // 2), :], BF16)
            r = jax.lax.dot_general(o_ref[:, pl.ds(g * G * Dh, G * Dh)], w,
                                    (((1,), (0,)), ((), ())), preferred_element_type=F32)
            if g == 0:
                acc_ref[...] = r
            elif g < H // G - 1:
                acc_ref[...] += r
            else:
                return acc_ref[...] + r

        s1, s2, s3 = cfg["skew_s"], cfg["skew_pv"], cfg["skew_wo"]
        res = None
        for t in range(H + s1 + s2 + s3):
            if t < H:
                proj(t)
            if 0 <= t - s1 < H:
                scores(t - s1)
            hh = t - s1 - s2
            if 0 <= hh < H:
                pv(hh)
            hw = t - s1 - s2 - s3
            if 0 <= hw < H and (hw + 1) % G == 0:
                res = wo_group(hw // G)
        mem_next = res[0:M, :].astype(BF16).astype(F32)
        b = res[M:L, :]
        g = jax.nn.sigmoid(jnp.sum(xs * gate_w, axis=-1, keepdims=True))
        a = xs * y_ref[pl.ds(r0, SEG), :]
        out_ref[pl.ds(r0, SEG), :] = (g * a + (1.0 - g) * b).astype(out_ref.dtype)
        pltpu.make_async_copy(out_ref.at[pl.ds(r0, SEG)], out_hbm.at[pl.ds(r0, SEG)], osem).start()
        return mem_next

    nst = cfg.get("nsteps", n_seg)
    jax.lax.fori_loop(0, nst, step, mem0_ref[...].astype(F32), unroll=cfg["su"])
    pltpu.make_async_copy(out_ref.at[0:nst * SEG], out_hbm.at[0:nst * SEG], osem).wait()


@functools.partial(jax.jit, static_argnames=("B_seg_len", "cfg"))
def pallas_gated_mix__ssm_conv_h3__memory_aug_recurrent_mem_tr__prompt_kernel(
    A_q, A_k, A_v, A_shift_k, A_ssm_k, A_ssm_D, B_x, B_mem0, B_Wq, B_Wk, B_Wv, B_Wo,
    B_seg_len, gate_w, cfg=None,
):
    del B_x
    cfg = dict(CFG, **dict(cfg or ()))
    _, S, D = A_q.shape
    _, H, Dh = B_Wq.shape
    M = B_mem0.shape[1]
    SEG = int(B_seg_len)
    L = M + SEG
    WD = cfg["WD"]
    NB = S // 128
    assert cfg["RI"] == 8
    consts = _dft_consts(2 * NB, 128, cfg["RI"])
    kern = functools.partial(_kernel, S, D, H, Dh, M, SEG, cfg)
    vm = pl.BlockSpec(memory_space=pltpu.VMEM)
    hbm = pl.BlockSpec(memory_space=pl.ANY)
    out = pl.pallas_call(
        kern,
        out_shape=jax.ShapeDtypeStruct((S, D), BF16),
        in_specs=[vm, vm, vm, vm] + [hbm] * 12,
        out_specs=hbm,
        scratch_shapes=[
            pltpu.VMEM((S, D), BF16),
            pltpu.VMEM((S, D), BF16),
            pltpu.VMEM((S, D), BF16),
            pltpu.VMEM((D, S), BF16),
            pltpu.VMEM((2 * NB, 128, 256), U32),
            pltpu.VMEM(consts[0].shape, F32),
            pltpu.VMEM(consts[1].shape, F32),
            pltpu.VMEM(consts[2].shape, F32),
            pltpu.VMEM((8, D), F32),
            pltpu.VMEM((2, S, WD), F32),
            pltpu.VMEM((2, S, WD), F32),
            pltpu.VMEM((2, NB, 128, 2 * WD), U32),
            pltpu.VMEM((2, 128, WD), U32),
            pltpu.VMEM((2, NB, 256, WD), F32),
            pltpu.VMEM((S, D), F32),
            pltpu.VMEM((3, D, H // 2, Dh), U32),
            pltpu.VMEM((D // 2, 3 * H * Dh), U32),
            pltpu.VMEM((H * Dh // 2, D), U32),
            pltpu.VMEM((L, D), F32),
            pltpu.VMEM((L, H * Dh), F32),
            pltpu.VMEM((L, D), F32),
            pltpu.VMEM((S, D), BF16),
            pltpu.SemaphoreType.DMA((3 * (D // WD) + 11,)),
            pltpu.SemaphoreType.DMA,
        ],
        compiler_params=pltpu.CompilerParams(
            vmem_limit_bytes=120 * 1024 * 1024, flags=dict(cfg["flags"]) or None),
    )(
        A_shift_k.T, A_ssm_D, B_mem0.reshape(M, D), gate_w,
        A_q.reshape(S, D), A_k.reshape(S, D), A_v.reshape(S, D), A_ssm_k,
        B_Wq, B_Wk, B_Wv, B_Wo.reshape(H * Dh, D), *consts,
    )
    return out.reshape(1, S, D)
```

```python
import functools
import math

import numpy as np
import jax
import jax.numpy as jnp
import jax.experimental.pallas as pl
import jax.experimental.pallas.tpu as pltpu

F32 = jnp.float32
BF16 = jnp.bfloat16
U32 = jnp.uint32

def _neg(a):
    return None if a is None else (-a[0], a[1])
def _add(a, b):
    if a is None or b is None:
        return b if a is None else a
    if a[0] == b[0]:
        return (a[0], a[1] + b[1])
    return (1, a[1] - b[1]) if a[0] > 0 else (1, b[1] - a[1])
def _sub(a, b):
    return _add(a, _neg(b))
def _val(a):
    return a[1] if a[0] > 0 else -a[1]
def _cadd(a, b): return (_add(a[0], b[0]), _add(a[1], b[1]))
def _csub(a, b): return (_sub(a[0], b[0]), _sub(a[1], b[1]))
def _mulc(a, c):
    if a is None or abs(c) < 1e-12: return None
    if abs(c - 1) < 1e-12: return a
    if abs(c + 1) < 1e-12: return _neg(a)
    return (1, a[1] * np.float32(c * a[0]))
def _ctw(z, num, den):
    num %= den
    re, im = z
    if (4 * num) % den == 0:
        qd = (4 * num) // den
        return [(re, im), (_neg(im), re), (_neg(re), _neg(im)), (im, _neg(re))][qd]
    c, s = math.cos(2 * math.pi * num / den), math.sin(2 * math.pi * num / den)
    if (8 * num) % den == 0 and re is not None and im is not None:
        if c * s > 0:
            return (_mulc(_sub(re, im), c), _mulc(_add(im, re), c))
        return (_mulc(_add(re, im), c), _mulc(_sub(im, re), c))
    return (_sub(_mulc(re, c), _mulc(im, s)), _add(_mulc(re, s), _mulc(im, c)))
def _cfft(zs, sign):
    n = len(zs)
    if n == 1: return list(zs)
    ev, od = _cfft(zs[0::2], sign), _cfft(zs[1::2], sign)
    out = [None] * n
    for j in range(n // 2):
        t = _ctw(od[j], sign * j, n)
        out[j] = _cadd(ev[j], t); out[j + n // 2] = _csub(ev[j], t)
    return out
def _conj(z): return (z[0], _neg(z[1]))
def rfft_sym(xs):
    n = len(xs)
    if n == 1: return [(xs[0], None)]
    if n == 2: return [(_add(xs[0], xs[1]), None), (_sub(xs[0], xs[1]), None)]
    hf, q = n // 2, n // 4
    s = [_add(xs[i], xs[i + hf]) for i in range(hf)]
    d = [_sub(xs[i], xs[i + hf]) for i in range(hf)]
    out = [None] * (hf + 1)
    for j, e in enumerate(rfft_sym(s)): out[2 * j] = e
    z = [_ctw((d[i], _neg(d[i + q])), -i, n) for i in range(q)]
    for j, e in enumerate(_cfft(z, -1)):
        m = 4 * j + 1
        if m <= hf: out[m] = e
        else: out[n - m] = _conj(e)
    return out
def irfft_sym(U, n, nout):
    if n == 1: return [U[0][0]]
    if n == 2: return [_add(U[0][0], U[1][0]), _sub(U[0][0], U[1][0])][:nout]
    hf, q = n // 2, n // 4
    e = irfft_sym(U[0::2], hf, hf)
    V = []
    for j in range(q):
        m = 4 * j + 1
        V.append(U[m] if m <= hf else _conj(U[n - m]))
    w = _cfft(V, +1)
    o = [None] * hf
    for i in range(q):
        t = _ctw(w[i], i, n)
        o[i] = t[0]; o[i + q] = _neg(t[1])
    y = [_add(e[i], o[i]) for i in range(hf)]
    if nout > hf: y += [_sub(e[i], o[i]) for i in range(hf)]
    return y[:nout]


def _bf16_bits(a):
    u = np.ascontiguousarray(a, np.float32).view(np.uint32)
    return (u + 0x7FFF + ((u >> 16) & 1)) >> 16


def _pack_rows(a):
    b = _bf16_bits(a)
    r = b.shape[0] // 2
    return (b[:r] | (b[r:] << 16)).astype(np.uint32)


@functools.lru_cache(maxsize=None)
def _dft_consts(N1, N2, RI):
    Lf, hN = N1 * N2, N2 // 2
    k2 = np.arange(N2)[:, None]
    n2 = np.arange(N2)[None, :]
    ph = -2 * np.pi * (k2 * n2 % N2) / N2
    Fr, Fi = np.cos(ph), np.sin(ph)
    Gr, Gi = Fr.T * (2.0 / Lf), -Fi.T * (2.0 / Lf)

    def inter(a, b):
        m = np.zeros((N2, 2 * N2))
        m[:, 0::2] = a; m[:, 1::2] = b
        return m
    base = np.stack([inter(Fr, -Fi), inter(Fi, Fr), inter(Gr, -Gi), inter(Gi, Gr)]).astype(np.float32)
    th = 2 * np.pi * np.arange(N1 // 2)[:, None] * np.arange(N2)[None, :] / Lf
    twf = np.stack([np.repeat(np.cos(th), 2, axis=1), np.repeat(np.sin(th), 2, axis=1)]).astype(np.float32)
    twg = np.zeros((N2, 128), np.float32)
    twg[:, :N1 // 2] = np.cos(th).T; twg[:, 64:64 + N1 // 2] = np.sin(th).T
    f = np.zeros((2 * N2, 2 * N2))
    g = np.zeros((2 * N2, 2 * N2))
    kk = np.arange(hN)[:, None]
    p0 = -2 * np.pi * (kk * n2 % N2) / N2
    p1 = -2 * np.pi * ((kk * n2 % N2) / N2 + n2 * (N1 // 2) / Lf)
    F0r, F0i, F1r, F1i = np.cos(p0), np.sin(p0), np.cos(p1), np.sin(p1)
    nyq = np.cos(np.pi * n2[0])
    f[:hN, 0::2] = F0r; f[hN:N2, 1::2] = F1r
    f[N2:N2 + hN, 0::2] = F0i; f[N2 + hN:, 1::2] = F1i
    f[N2, 0::2] = nyq
    c = 2.0 / Lf
    g[:N2, 0:N2:2] = F0r.T * c; g[:N2, 1:N2:2] = F0i.T * c
    g[:N2, 0] = 1.0 / Lf; g[:N2, 1] = nyq / Lf
    g[N2:, N2::2] = F1r.T * c; g[N2:, N2 + 1::2] = F1i.T * c
    perm = np.arange(2 * N2).reshape(2, N2 // RI, RI).transpose(1, 0, 2).reshape(-1)
    sp = np.stack([_pack_rows(f[perm]), _pack_rows(g)])
    return base, twf, twg, sp


CFG = dict(G=1, skew_s=1, skew_pv=5, skew_wo=4, WD=256, RI=8, MS=128, MS2=128, order="21AIRK", unroll=1, su=4,
           slots=((0, (("unroll", 2),)), (1, (("unroll", 2),)),
                  (2, (("MS", 256), ("MS2", 256))),
                  (5, (("unroll", 2), ("order", "12IAKR")))))


def _kernel(S, D, H, Dh, M, SEG, cfg,
            shift_ref, ssmD_ref, mem0_ref, gatew_ref,
            q_hbm, k_hbm, v_hbm, ssmk_hbm, wq_hbm, wk_hbm, wv_hbm, wo_hbm, cb_hbm, ctf_hbm, ctg_hbm, csp_hbm,
            out_hbm,
            x_ref, k_ref, v_ref, ssm_ref, tab_ref, cb_ref, ctf_ref, ctg_ref, shT, kv_s, hT_s, A_s, Y_s, U_s, y_ref,
            wraw, wqkv, wo, h_ref, o_ref, acc_ref, out_ref, sems, osem):
    L = M + SEG
    n_seg = S // SEG
    HP = H // 2
    WD, RI = cfg["WD"], cfg["RI"]
    N2 = 128
    NB = S // N2
    NL = WD // 128
    NBLK = D // WD

    def cp_blk(b):
        ls = pl.ds(b * WD, WD)
        return [pltpu.make_async_copy(k_hbm.at[:, ls], k_ref.at[:, ls], sems.at[3 * b]),
                pltpu.make_async_copy(v_hbm.at[:, ls], v_ref.at[:, ls], sems.at[3 * b + 1]),
                pltpu.make_async_copy(ssmk_hbm.at[ls, :], ssm_ref.at[ls, :], sems.at[3 * b + 2])]

    def wraw_copy(src, slot, sem):
        return pltpu.make_async_copy(src.bitcast(U32), wraw.at[slot], sems.at[sem])

    s0 = 3 * NBLK
    cp_c = [pltpu.make_async_copy(cb_hbm, cb_ref, sems.at[s0]),
            pltpu.make_async_copy(ctf_hbm, ctf_ref, sems.at[s0 + 1]),
            pltpu.make_async_copy(ctg_hbm, ctg_ref, sems.at[s0 + 8]),
            pltpu.make_async_copy(csp_hbm.at[0], tab_ref.at[0], sems.at[s0 + 9]),
            pltpu.make_async_copy(csp_hbm.at[1], tab_ref.at[NB], sems.at[s0 + 10])]
    cp_w = [wraw_copy(w, i, s0 + 2 + i) for i, w in enumerate((wq_hbm, wk_hbm, wv_hbm))]
    cp_wo = pltpu.make_async_copy(wo_hbm.bitcast(U32), wo, sems.at[s0 + 5])
    cp_x = pltpu.make_async_copy(q_hbm, x_ref, sems.at[s0 + 6])
    blk_cps = [cp_blk(b) for b in range(NBLK)]
    for c in cp_c:
        c.start()
    for b in range(NBLK):
        for c in blk_cps[b]:
            c.start()
    for c in cp_w + [cp_wo, cp_x]:
        c.start()

    ks_taps = shift_ref.shape[0]
    shT[0:ks_taps, :] = shift_ref[...].astype(F32)
    shT[ks_taps:ks_taps + 1, :] = ssmD_ref[...].astype(F32).reshape(1, D)
    eye = (jax.lax.broadcasted_iota(jnp.int32, (N2, N2), 0)
           == jax.lax.broadcasted_iota(jnp.int32, (N2, N2), 1)).astype(BF16)

    for c in cp_c:
        c.wait()
    hq = N2 // 2
    for k1 in range(1, NB):
        cf, sf = ctf_ref[0, k1:k1 + 1, :], ctf_ref[1, k1:k1 + 1, :]
        for q in range(N2 // 8):
            g8 = (q // 2) * 8

            def rot(r):
                fre, fim = cb_ref[0, r:r + 8, :], cb_ref[1, r:r + 8, :]
                return fre * cf + fim * sf if q % 2 == 0 else fim * cf - fre * sf
            tab_ref[k1, q * 8:q * 8 + 8, :] = pltpu.pack_elementwise([rot(g8), rot(hq + g8)], packed_dtype=BF16)
            rows = slice(q * 8, q * 8 + 8)
            cg = jnp.broadcast_to(ctg_ref[rows, k1:k1 + 1], (8, 2 * N2))
            sg = jnp.broadcast_to(ctg_ref[rows, 64 + k1:64 + k1 + 1], (8, 2 * N2))
            gre, gim = cb_ref[2, rows, :], cb_ref[3, rows, :]
            tab_ref[NB + k1, rows, :] = pltpu.pack_elementwise(
                [gre * cg - gim * sg, gim * cg + gre * sg], packed_dtype=BF16)

    def st_kv(b, i):
        r0 = pl.multiple_of(i * N2, N2)
        rp = pl.multiple_of(jnp.maximum(r0 - 16, 0), 16)
        for j in range(NL):
            lg = pl.ds(b * WD + j * 128, 128)
            ll = pl.ds(j * 128, 128)
            cur = k_ref[pl.ds(r0, N2), lg].astype(F32)
            prev = jnp.where(i > 0, k_ref[pl.ds(rp, 16), lg].astype(F32), 0.0)
            ext = jnp.concatenate([prev[8:16], cur], axis=0)
            w = shT[0:ks_taps + 1, lg]
            ks = cur * w[0:1]
            for t in range(1, ks_taps):
                ks = ks + ext[8 - t:8 - t + N2] * w[t:t + 1]
            kv = ks * v_ref[pl.ds(r0, N2), lg].astype(F32)
            kv_s[b % 2, pl.ds(r0, N2), ll] = kv
            y_ref[pl.ds(r0, N2), lg] = kv * w[ks_taps:ks_taps + 1]
            hT_s[b % 2, pl.ds(r0, N2), ll] = jax.lax.dot_general(
                eye, ssm_ref[lg, pl.ds(r0, N2)], (((1,), (1,)), ((), ())), preferred_element_type=F32)
            yield

    def st_a(b, i):
        r0 = pl.multiple_of(i * 8, 8)
        for src, off in ((kv_s, 0), (hT_s, 128)):
            for j in range(NL):
                xs = [src[b % 2, pl.ds(n1 * N2 + r0, 8), pl.ds(j * 128, 128)] for n1 in range(NB)]
                X = rfft_sym([(1, x) for x in xs] + [None] * NB)
                for k1 in range(NB):
                    pair = [X[0][0], X[NB][0]] if k1 == 0 else [X[k1][0], X[k1][1]]
                    pair = [_val(t) for t in pair]
                    A_s[b % 2, k1, pl.ds(r0, 8), pl.ds(off + j * 256, 128)] = (
                        pltpu.pack_elementwise(pair, packed_dtype=BF16))
                yield

    def table(idx):
        w = tab_ref[idx]
        return jnp.concatenate([pltpu.bitcast(w << 16, F32),
                                pltpu.bitcast(w & np.uint32(0xFFFF0000), F32)], axis=0)

    def mm(a, b):
        return jax.lax.dot_general(a, b, (((1,), (0,)), ((), ())), preferred_element_type=F32)

    def st_g1(b, i, par):
        Fm = table(i)
        MS = cfg["MS"]
        for j in range(NL):
            Am = pltpu.bitcast(A_s[b % 2, i, :, pl.ds(j * 256, 256)], BF16)
            for m0 in range(0, 2 * N2, MS):
                X = mm(Fm[m0:m0 + MS], Am)
                for r in range(MS // (2 * RI)):
                    re = X[2 * r * RI:(2 * r + 1) * RI]
                    im = X[(2 * r + 1) * RI:(2 * r + 2) * RI]
                    a, c = re[:, :128], re[:, 128:]
                    b_, d = im[:, :128], im[:, 128:]
                    bd = b_ * d
                    yre, yim = a * c - bd, a * d + b_ * c
                    row = m0 // 2 + r * RI
                    if row == 0:
                        rid = jax.lax.broadcasted_iota(jnp.int32, (RI, 128), 0) + i
                        yre = jnp.where(rid == 0, a * c, yre)
                        yim = jnp.where(rid == 0, bd, yim)
                    Y_s[par, pl.ds(row, RI), pl.ds(j * 128, 128)] = (
                        pltpu.pack_elementwise([yre, yim], packed_dtype=BF16))
                yield

    def st_g2(b, i, par):
        Gm = table(NB + i)
        MS = cfg["MS2"]
        Ym = pltpu.bitcast(Y_s[par], BF16)
        for m0 in range(0, 2 * N2, MS):
            U_s[b % 2, i, pl.ds(m0, MS), :] = mm(Gm[m0:m0 + MS], Ym)
            yield

    def st_i(b, i):
        r0 = pl.multiple_of(i * 8, 8)
        for j in range(NL):
            lg = pl.ds(b * WD + j * 128, 128)
            ld = lambda k1, part: (1, U_s[b % 2, k1, pl.ds(part * N2 + r0, 8), pl.ds(j * 128, 128)])
            U = [(ld(0, 0), None)] + [(ld(k1, 0), ld(k1, 1)) for k1 in range(1, NB)] + [(ld(0, 1), None)]
            ys = irfft_sym(U, 2 * NB, NB)
            for n1 in range(NB):
                rr = pl.ds(n1 * N2 + r0, 8)
                y_ref[rr, lg] = _val(_add((1, y_ref[rr, lg]), ys[n1]))
            yield

    def st_relayout(slot, i, n_per):
        for u in range(n_per):
            ii = i * n_per + u
            r0 = pl.multiple_of(ii * 8, 8)
            raw = wraw.at[slot].reshape(D * HP, Dh)
            for hp in range(HP):
                a = raw[pl.ds(ii * 16 * HP + hp, 8, stride=2 * HP), :]
                b = raw[pl.ds(ii * 16 * HP + HP + hp, 8, stride=2 * HP), :]
                c0 = (2 * hp) * 3 * Dh + slot * Dh
                wqkv[pl.ds(r0, 8), pl.ds(c0, Dh)] = (a & 0xFFFF) | (b << 16)
                wqkv[pl.ds(r0, 8), pl.ds(c0 + 3 * Dh, Dh)] = (a >> 16) | (b & np.uint32(0xFFFF0000))
            yield

    rel_slot = cfg.get("rel_slot", (NBLK - 1, NBLK, NBLK + 1))
    n_slots = max(NBLK + 3, max(rel_slot) + 1)
    cfg = dict(cfg)
    cfg0 = dict(cfg)
    for slot in range(n_slots):
        cfg.update(cfg0)
        cfg.update(dict(dict(cfg0["slots"]).get(slot, ())))
        bk, ba, bg, bi = slot, slot - 1, slot - 2, slot - 3
        ok = lambda b: 0 <= b < NBLK
        if ok(bk):
            for c in blk_cps[bk]:
                c.wait()
        rel = [m for m in range(3) if rel_slot[m] == slot]
        for m in rel:
            cp_w[m].wait()

        def body1(i, par, first=False, bk=bk, ba=ba, bg=bg, bi=bi, rel=rel):
            gens = []
            for st in cfg["order"]:
                if st == "1" and ok(bg):
                    gens.append(st_g1(bg, i, par))
                elif st == "2" and ok(bg) and not first:
                    gens.append(st_g2(bg, i - 1, 1 - par))
            for st in cfg["order"]:
                if st == "I" and ok(bi):
                    gens.append(st_i(bi, i))
                elif st == "A" and ok(ba):
                    gens.append(st_a(ba, i))
                elif st == "K" and ok(bk):
                    gens.append(st_kv(bk, i))
                elif st == "R":
                    gens.extend(st_relayout(m, i, D // 16 // NB) for m in rel)
            for g_ in gens:
                for _ in g_:
                    pass

        UN = cfg["unroll"]

        def body(i0, carry):
            for u in range(UN):
                body1(i0 * UN + u, u % 2 if UN > 1 else (i0 % 2))
            return carry

        if ok(bg):
            for u in range(UN):
                body1(u, u % 2, first=(u == 0))
            jax.lax.fori_loop(1, NB // UN, body, 0)
            for _ in st_g2(bg, NB - 1, (NB - 1) % 2):
                pass
        else:
            jax.lax.fori_loop(0, NB // UN, body, 0)

    cfg.update(cfg0)
    cp_wo.wait()
    cp_x.wait()

    scale = Dh ** (-0.5)
    G = cfg["G"]
    gate_w = gatew_ref[...].astype(F32).reshape(1, D)

    def step(s, mem):
        r0 = pl.multiple_of(s * SEG, SEG)
        xs = x_ref[pl.ds(r0, SEG), :].astype(F32)
        h_ref[0:M, :] = mem
        h_ref[M:L, :] = xs
        row = jax.lax.broadcasted_iota(jnp.int32, (L, L), 0)
        col = jax.lax.broadcasted_iota(jnp.int32, (L, L), 1)
        mask = (row < M) | (row >= col)

        qkv = {}
        probs = {}

        def proj(h):
            w = pltpu.bitcast(wqkv[:, pl.ds(h * 3 * Dh, 3 * Dh)], BF16)
            r = jax.lax.dot_general(h_ref[...], w, (((1,), (0,)), ((), ())),
                                    preferred_element_type=F32)
            qkv[h] = (r[:, :Dh], r[:, Dh:2 * Dh].astype(BF16), r[:, 2 * Dh:].astype(BF16))

        def scores(h):
            q, k, _ = qkv[h]
            sc = jax.lax.dot_general(q, k, (((1,), (1,)), ((), ())),
                                     preferred_element_type=F32) * scale
            sc = jnp.where(mask, sc, -1e9)
            m = jnp.max(sc, axis=-1, keepdims=True)
            e = jnp.exp(sc - m)
            probs[h] = e / jnp.sum(e, axis=-1, keepdims=True)

        def pv(h):
            o = jax.lax.dot_general(probs.pop(h), qkv.pop(h)[2], (((1,), (0,)), ((), ())),
                                    preferred_element_type=F32)
            o_ref[:, pl.ds(h * Dh, Dh)] = o

        def wo_group(g):
            w = pltpu.bitcast(wo[pl.ds(g * G * Dh // 2, G * Dh // 2), :], BF16)
            r = jax.lax.dot_general(o_ref[:, pl.ds(g * G * Dh, G * Dh)], w,
                                    (((1,), (0,)), ((), ())), preferred_element_type=F32)
            if g == 0:
                acc_ref[...] = r
            elif g < H // G - 1:
                acc_ref[...] += r
            else:
                return acc_ref[...] + r

        s1, s2, s3 = cfg["skew_s"], cfg["skew_pv"], cfg["skew_wo"]
        res = None
        for t in range(H + s1 + s2 + s3):
            if t < H:
                proj(t)
            if 0 <= t - s1 < H:
                scores(t - s1)
            hh = t - s1 - s2
            if 0 <= hh < H:
                pv(hh)
            hw = t - s1 - s2 - s3
            if 0 <= hw < H and (hw + 1) % G == 0:
                res = wo_group(hw // G)
        mem_next = res[0:M, :].astype(BF16).astype(F32)
        b = res[M:L, :]
        g = jax.nn.sigmoid(jnp.sum(xs * gate_w, axis=-1, keepdims=True))
        a = xs * y_ref[pl.ds(r0, SEG), :]
        out_ref[pl.ds(r0, SEG), :] = (g * a + (1.0 - g) * b).astype(out_ref.dtype)
        pltpu.make_async_copy(out_ref.at[pl.ds(r0, SEG)], out_hbm.at[pl.ds(r0, SEG)], osem).start()
        return mem_next

    jax.lax.fori_loop(0, n_seg, step, mem0_ref[...].astype(F32), unroll=cfg["su"])
    pltpu.make_async_copy(out_ref, out_hbm, osem).wait()


@functools.partial(jax.jit, static_argnames=("B_seg_len", "cfg"))
def pallas_gated_mix__ssm_conv_h3__memory_aug_recurrent_mem_tr__prompt_kernel(
    A_q, A_k, A_v, A_shift_k, A_ssm_k, A_ssm_D, B_x, B_mem0, B_Wq, B_Wk, B_Wv, B_Wo,
    B_seg_len, gate_w, cfg=None,
):
    del B_x
    cfg = dict(CFG, **dict(cfg or ()))
    _, S, D = A_q.shape
    _, H, Dh = B_Wq.shape
    M = B_mem0.shape[1]
    SEG = int(B_seg_len)
    L = M + SEG
    WD = cfg["WD"]
    NB = S // 128
    assert cfg["RI"] == 8
    consts = _dft_consts(2 * NB, 128, cfg["RI"])
    kern = functools.partial(_kernel, S, D, H, Dh, M, SEG, cfg)
    vm = pl.BlockSpec(memory_space=pltpu.VMEM)
    hbm = pl.BlockSpec(memory_space=pl.ANY)
    out = pl.pallas_call(
        kern,
        out_shape=jax.ShapeDtypeStruct((S, D), BF16),
        in_specs=[vm, vm, vm, vm] + [hbm] * 12,
        out_specs=hbm,
        scratch_shapes=[
            pltpu.VMEM((S, D), BF16),
            pltpu.VMEM((S, D), BF16),
            pltpu.VMEM((S, D), BF16),
            pltpu.VMEM((D, S), BF16),
            pltpu.VMEM((2 * NB, 128, 256), U32),
            pltpu.VMEM(consts[0].shape, F32),
            pltpu.VMEM(consts[1].shape, F32),
            pltpu.VMEM(consts[2].shape, F32),
            pltpu.VMEM((8, D), F32),
            pltpu.VMEM((2, S, WD), F32),
            pltpu.VMEM((2, S, WD), F32),
            pltpu.VMEM((2, NB, 128, 2 * WD), U32),
            pltpu.VMEM((2, 128, WD), U32),
            pltpu.VMEM((2, NB, 256, WD), F32),
            pltpu.VMEM((S, D), F32),
            pltpu.VMEM((3, D, H // 2, Dh), U32),
            pltpu.VMEM((D // 2, 3 * H * Dh), U32),
            pltpu.VMEM((H * Dh // 2, D), U32),
            pltpu.VMEM((L, D), F32),
            pltpu.VMEM((L, H * Dh), F32),
            pltpu.VMEM((L, D), F32),
            pltpu.VMEM((S, D), BF16),
            pltpu.SemaphoreType.DMA((3 * (D // WD) + 11,)),
            pltpu.SemaphoreType.DMA,
        ],
        compiler_params=pltpu.CompilerParams(vmem_limit_bytes=120 * 1024 * 1024),
    )(
        A_shift_k.T, A_ssm_D, B_mem0.reshape(M, D), gate_w,
        A_q.reshape(S, D), A_k.reshape(S, D), A_v.reshape(S, D), A_ssm_k,
        B_Wq, B_Wk, B_Wv, B_Wo.reshape(H * Dh, D), *consts,
    )
    return out.reshape(1, S, D)
```
